```python
import jax
import jax.numpy as jnp

def _softmax(x, axis=-1):
    return jax.nn.softmax(x, axis=axis)
def _gelu(x):
    return jax.nn.gelu(x, approximate=True)
def _silu(x):
    return jax.nn.silu(x)
def _sigmoid(x):
    return jax.nn.sigmoid(x)
def _layernorm(x, axis=-1, eps=1e-5):
    m = jnp.mean(x, axis=axis, keepdims=True)
    v = jnp.var(x, axis=axis, keepdims=True)
    return (x - m) / jnp.sqrt(v + eps)
def _scatter_add(tgt, idx, src, axis=0):
    return tgt.at[idx].add(src)
def _segment_sum(src, seg, n):
    return jax.ops.segment_sum(src, seg, n)
class _Rng:
    def __init__(self, key):
        self._k = key
    def _next(self):
        self._k, sub = jax.random.split(self._k)
        return sub
    def normal(self, shape):
        return jax.random.normal(self._next(), shape, dtype=jnp.bfloat16)
    def randint(self, lo, hi, shape):
        return jax.random.randint(self._next(), shape, lo, hi, dtype=jnp.int32)
    def uniform(self, shape, lo=0.0, hi=1.0):
        return jax.random.uniform(self._next(), shape, jnp.bfloat16, lo, hi)
    def permutation(self, n):
        return jax.random.permutation(self._next(), n)


kernel_name = 'standalone__structured_sparse_n_m__ragged'

def setup_inputs():
    _rng = _Rng(jax.random.key(int.from_bytes(__import__("os").urandom(4), "little")))
    _w = (lambda a: (lambda t: t.astype(jnp.bfloat16) if jnp.issubdtype(t.dtype, jnp.floating) else t)(jnp.asarray(a)))
    B, S, D = 16, 4096, 576
    assert D % 4 == 0, "d_model must be divisible by M=4 for 2:4 sparsity"
    return {
        "x": _w((lambda *s: _rng.normal(s) * 0.05)(B, S, D)),
        "w": _w((lambda *s: _rng.normal(s) * 0.05)(D, D)),
        "b": _w((lambda *s: _rng.normal(s) * 0.05)(D)),
    }

def reference(x, w, b):
    B, S, D = x.shape
    N, M = 2, 4
    G = D // M
    wg = w.reshape(G, M, D)
    mag = jnp.abs(wg)
    order = jnp.argsort(mag, 1)
    thr = jnp.take_along_axis(mag, order[:, M - N:M - N + 1, :], 1)
    mask = (lambda x, dt: x.astype(dt))(mag >= thr, w.dtype)
    wp = (wg * mask).reshape(D, D)
    return jnp.einsum("bsd,df->bsf", x, wp) + b
```

```python
import jax
import jax.numpy as jnp
from jax import lax
import jax.experimental.pallas as pl
import jax.experimental.pallas.tpu as pltpu

KU = 64
PAIR = 256
WC = 512
SHIFT = 3
OUT_SLOTS = 9
IN_FIRST = (256, 256, 512, 1024, 2048)

_T = 1.0 / 3.0
_SCHEME = (
    (({(0, 0): 1, (0, 1): -1},
      ({(0, 0): 1, (0, 1): -1}, {(1, 1): 1}), ({(0, 6): 1, (0, 7): -1}, {(7, 1): 1})),
     ({(0, 0): 1, (0, 1): -.5},
      ({(0, 2): 2, (0, 3): -2}, {(3, 1): 1}), ({(0, 4): 2, (0, 5): -2}, {(5, 1): 1})),
     ({(1, 0): 1, (1, 1): -1},
      ({(1, 0): 1, (1, 1): -1}, {(0, 0): 1}), ({(1, 6): 1, (1, 7): -1}, {(6, 0): 1})),
     ({(1, 0): 1, (1, 1): -.5},
      ({(1, 2): 1, (1, 3): -1}, {(2, 0): 1}), ({(1, 4): 1, (1, 5): -1}, {(4, 0): 1}))),
    (({(0, 0): 1, (1, 1): 1},
      ({(0, 0): 1, (1, 1): -1}, {(0, 0): 1, (1, 1): -1}),
      ({(0, 2): 1, (1, 3): -.5}, {(2, 0): 1, (3, 1): -2})),
     ({(0, 0): 1, (1, 1): .5},
      ({(0, 4): 1, (1, 5): -1}, {(4, 0): 1, (5, 1): -2}),
      ({(0, 6): 1, (1, 7): -2}, {(6, 0): 1, (7, 1): -1})),
     ({(0, 0): 1},
      ({(0, 1): 1, (1, 1): -1}, {(1, 0): 1, (1, 1): 1}),
      ({(0, 3): 1, (1, 3): -.5}, {(3, 0): 1, (3, 1): 2})),
     ({(1, 1): 1},
      ({(0, 0): -1, (1, 0): 1}, {(0, 0): 1, (0, 1): 1}),
      ({(0, 2): -1, (1, 2): .5}, {(2, 0): 1, (2, 1): 2}))),
    (({(0, 0): 1, (1, 0): 1},
      ({(1, 1): 1}, {(0, 0): 1, (1, 0): 1}), ({(1, 5): 1}, {(4, 0): 1, (5, 0): 1})),
     ({(0, 0): 1, (1, 0): 2},
      ({(1, 3): .5}, {(2, 0): 1, (3, 0): 1}), ({(0, 8): -_T, (1, 8): 2 * _T}, {(8, 0): 1})),
     ({(0, 0): 1, (1, 0): .5},
      ({(1, 7): 2}, {(6, 0): 1, (7, 0): 1}), ({(0, 8): 4 * _T, (1, 8): -2 * _T}, {(8, 0): 1})),
     ({(0, 0): 1},
      ({(0, 5): 1, (1, 5): -1}, {(5, 0): 1, (5, 1): 2}),
      ({(0, 7): 1, (1, 7): -2}, {(7, 0): 1, (7, 1): 1}))),
    (({(0, 1): 1, (1, 1): 1},
      ({(0, 0): 1}, {(0, 1): 1, (1, 1): 1}), ({(0, 4): 1}, {(4, 1): 1, (5, 1): 1})),
     ({(0, 1): 1, (1, 1): 2},
      ({(0, 2): 1}, {(2, 1): 1, (3, 1): 1}), ({(0, 8): -_T, (1, 8): 2 * _T}, {(8, 1): 1})),
     ({(0, 1): 1, (1, 1): .5},
      ({(0, 6): 1}, {(6, 1): 1, (7, 1): 1}), ({(0, 8): 4 * _T, (1, 8): -2 * _T}, {(8, 1): 1})),
     ({(1, 1): 1},
      ({(0, 4): -.5, (1, 4): .5}, {(4, 0): 1, (4, 1): 2}),
      ({(0, 6): -.5, (1, 6): 1}, {(6, 0): 1, (6, 1): 1}))),
)


def _lincomb(terms, acc=None):
    for mag in sorted({abs(c) for c, _ in terms}, key=lambda m: (m != 1, m)):
        grp = sorted([(c, v) for c, v in terms if abs(c) == mag], key=lambda t: -t[0])
        if mag == 1 and acc is not None:
            for c, v in grp:
                acc = acc + v if c > 0 else acc - v
            continue
        sgn = 1 if grp[0][0] > 0 else -1
        s = grp[0][1]
        for c, v in grp[1:]:
            s = s + v if c * sgn > 0 else s - v
        if mag != 1:
            s = s * mag
        if acc is None:
            acc = s if sgn > 0 else -s
        else:
            acc = acc + s if sgn > 0 else acc - s
    return acc


def _prune_packed(u):
    mate = lax.broadcasted_iota(jnp.int32, u.shape, 0) ^ 1
    lo = pltpu.bitcast((u << 16) & 0x7FFFFFFF, jnp.float32)
    hi = pltpu.bitcast(u & 0x7FFF0000, jnp.float32)
    big, small = jnp.maximum(lo, hi), jnp.minimum(lo, hi)
    nbig = jnp.take_along_axis(big, mate, axis=0, mode="promise_in_bounds")
    nsmall = jnp.take_along_axis(small, mate, axis=0, mode="promise_in_bounds")
    thr = jnp.maximum(jnp.minimum(big, nbig), jnp.maximum(small, nsmall))
    return u & (jnp.where(lo < thr, 0, 0xFFFF) | jnp.where(hi < thr, 0, -65536))


def _half(v, i, nk):
    n = v.shape[0] // nk
    return jnp.concatenate(
        [v[n * k + i * n // 2:n * k + (i + 1) * n // 2] for k in range(nk)], axis=0)


def _prepare_weights(wbuf, a_ref):
    nk = wbuf.shape[0] // KU
    u = pltpu.bitcast(wbuf[...], jnp.int32)
    wp = jnp.concatenate(
        [_prune_packed(u[r:r + 8]) for r in range(0, u.shape[0], 8)], axis=0)
    tiles = {}

    def tile(k0, k1):
        if (k0, k1) not in tiles:
            t = jnp.concatenate([wp[KU // 2 * k:KU // 2 * (k + 1)] for k in (k0, k1)], axis=0)
            tiles[k0, k1] = pltpu.bitcast(pltpu.bitcast(t, jnp.bfloat16).T, jnp.int32)
        return tiles[k0, k1]

    lane = lax.broadcasted_iota(jnp.int32, (1, 128), 1)
    for p, (_, (a0, _), (a1, _)) in enumerate(q for rnd in _SCHEME for q in rnd):
        acc = None
        for i in range(2):
            s0 = [k for k in sorted(a0) if k[0] == i]
            s1 = [k for k in sorted(a1) if k[0] == i]
            for q in range(max(len(s0), len(s1))):
                k0, c0 = (s0[q], a0[s0[q]]) if q < len(s0) else (min(a0), 0.0)
                k1, c1 = (s1[q], a1[s1[q]]) if q < len(s1) else (min(a1), 0.0)
                t = pltpu.bitcast(_half(tile(k0[1], k1[1]), i, nk), jnp.bfloat16)
                v = t.astype(jnp.float32)
                if not c0 == c1 == 1:
                    v = v * jnp.where(lane < KU, c0, c1)
                acc = v if acc is None else acc + v
        a_ref[p] = pltpu.bitcast(acc.astype(jnp.bfloat16), jnp.int32)


def _compute_pair(xbuf, obuf, a_ref, bias_ref, b, slot, o):
    nk = obuf.shape[1]
    xs = {}

    def xblk(k, j):
        if (k, j) not in xs:
            xs[k, j] = xbuf[b, k, :, pl.ds(o + 128 * j, 128)]
        return xs[k, j]

    def rhs(b0, b1):
        if len(b0) == len(b1) == 1:
            return jnp.concatenate([xblk(*min(b0)), xblk(*min(b1))], axis=0)
        parts = [_lincomb([(c, xblk(*k).astype(jnp.float32)) for k, c in t.items()])
                 for t in (b0, b1)]
        return jnp.concatenate(parts, axis=0).astype(jnp.bfloat16)

    last = {c: n for n, rnd in enumerate(_SCHEME) for q in rnd for c in q[0]}
    acc = {}
    for n, rnd in enumerate(_SCHEME):
        m = [jnp.dot(pltpu.bitcast(a_ref[4 * n + q], jnp.bfloat16), rhs(b0, b1),
                     preferred_element_type=jnp.float32)
             for q, (_, (_, b0), (_, b1)) in enumerate(rnd)]
        for c in sorted(last):
            terms = [(q[0][c], v) for q, v in zip(rnd, m) if c in q[0]]
            if not terms:
                continue
            acc[c] = _lincomb(terms, acc[c] if c in acc else bias_ref[c[0]])
            if last[c] == n:
                obuf[slot, :, pl.ds(KU // 2 * c[0], KU // 2), pl.ds(o + 128 * c[1], 128)] = (
                    acc[c].astype(obuf.dtype).reshape(nk, KU // 2, 128))


def _kernel(x_hbm, w_hbm, b_hbm, o_hbm,
            xbuf, obuf, wbuf, bbuf, a_ref, bias_ref, isem, fsem, osem, wsem):
    NB, NK, _, S = x_hbm.shape
    F = w_hbm.shape[1]
    first = [(sum(IN_FIRST[:j]), n) for j, n in enumerate(IN_FIRST)]

    def icopy(b):
        return pltpu.make_async_copy(x_hbm.at[b], xbuf.at[b], isem.at[b])

    def fcopy(j):
        cols = pl.ds(*first[j])
        return pltpu.make_async_copy(
            x_hbm.at[0, :, :, cols], xbuf.at[0, :, :, cols], fsem.at[j])

    def oslot(b):
        return jnp.where(b >= OUT_SLOTS, b - OUT_SLOTS, b)

    def ostart(b, o, n):
        for r in range(0, KU, 8):
            pltpu.make_async_copy(
                obuf.at[oslot(b), :, pl.ds(r, 8), pl.ds(o, n)],
                o_hbm.at[b, :, pl.ds(r, 8), pl.ds(o, n)], osem.at[b]).start()

    def owait(b):
        pltpu.make_async_copy(obuf.at[oslot(b)], o_hbm.at[b], osem.at[b]).wait()

    wcp = pltpu.make_async_copy(w_hbm, wbuf, wsem.at[0])
    bcp = pltpu.make_async_copy(b_hbm, bbuf, wsem.at[1])
    bcp.start()
    wcp.start()
    for j in range(len(first)):
        fcopy(j).start()
    for b in range(1, NB):
        icopy(b).start()

    bcp.wait()
    bias = jnp.broadcast_to(bbuf[...].reshape(1, F).astype(jnp.float32), (128, F)).T
    for i in range(2):
        bias_ref[i] = _half(bias, i, NK)
    wcp.wait()
    _prepare_weights(wbuf, a_ref)

    G = S // WC
    NP = S // PAIR
    assert NP == 2 * G
    late = [g for g in range(G) if (g + 1) * WC > PAIR * (G + g - SHIFT + 1)]

    @pl.loop(0, NB)
    def _(i):
        @pl.when(i > 0)
        def _():
            icopy(i).wait()

        @pl.when(i >= OUT_SLOTS)
        def _():
            owait(i - OUT_SLOTS)

        slot = oslot(i)
        for p in range(NP):
            for j, (o, _) in enumerate(first):
                if o == PAIR * p:
                    @pl.when(i == 0)
                    def _():
                        fcopy(j).wait()

            _compute_pair(xbuf, obuf, a_ref, bias_ref, i, slot, PAIR * p)

            db, g = divmod(p + SHIFT, G)
            b = 2 * i - NB + db
            in_last = db == 0 or (db == 1 and g not in late)

            @pl.when((b >= 0) & (i < (NB if in_last else NB - 1)))
            def _():
                ostart(b, g * WC, WC)

            if p * PAIR // WC in late and p < NP - 1:
                @pl.when(i == NB - 1)
                def _():
                    ostart(NB - 1, PAIR * p, PAIR)

    ostart(NB - 1, S - PAIR, PAIR)
    for b in range(NB - OUT_SLOTS, NB):
        owait(b)


@jax.jit
def pallas_standalone__structured_sparse_n_m__ragged_kernel(
    x: jax.Array,
    w: jax.Array,
    b: jax.Array,
):
    B, S, D = x.shape
    F = w.shape[1]
    xt = jnp.transpose(x, (0, 2, 1)).reshape(B, D // KU, KU, S)
    out = pl.pallas_call(
        _kernel,
        in_specs=[pl.BlockSpec(memory_space=pl.ANY)] * 3,
        out_specs=pl.BlockSpec(memory_space=pl.ANY),
        out_shape=jax.ShapeDtypeStruct((B, F // KU, KU, S), x.dtype),
        scratch_shapes=[
            pltpu.VMEM((B, D // KU, KU, S), x.dtype),
            pltpu.VMEM((OUT_SLOTS, F // KU, KU, S), x.dtype),
            pltpu.VMEM((D, F), w.dtype),
            pltpu.VMEM((F,), b.dtype),
            pltpu.VMEM((16, F // 4, 128), jnp.int32),
            pltpu.VMEM((2, F // 2, 128), jnp.float32),
            pltpu.SemaphoreType.DMA((B,)),
            pltpu.SemaphoreType.DMA((len(IN_FIRST),)),
            pltpu.SemaphoreType.DMA((B,)),
            pltpu.SemaphoreType.DMA((2,)),
        ],
        compiler_params=pltpu.CompilerParams(
            vmem_limit_bytes=122 * 1024 * 1024,
            disable_bounds_checks=True,
            flags={"XLA_TPU_RESCHEDULE_DMA_DONES": True},
        ),
    )(xt, w, b)
    return jnp.transpose(out.reshape(B, F, S), (0, 2, 1))
```

```python
import jax
import jax.numpy as jnp
from jax import lax
import jax.experimental.pallas as pl
import jax.experimental.pallas.tpu as pltpu

KU = 64
PAIR = 256
OUT_SLOTS = 9

_T = 1.0 / 3.0
_PLAIN = (
    (({(0, 0): 1, (0, 1): -1},
      ({(0, 0): 1, (0, 1): -1}, {(1, 1): 1}), ({(0, 6): 1, (0, 7): -1}, {(7, 1): 1})),
     ({(0, 0): 1, (0, 1): -.5},
      ({(0, 4): 2, (0, 5): -2}, {(5, 1): 1}), ({(0, 2): 2, (0, 3): -2}, {(3, 1): 1})),
     ({(1, 0): 1, (1, 1): -1},
      ({(1, 0): 1, (1, 1): -1}, {(0, 0): 1}), ({(1, 6): 1, (1, 7): -1}, {(6, 0): 1})),
     ({(1, 0): 1, (1, 1): -.5},
      ({(1, 4): 1, (1, 5): -1}, {(4, 0): 1}), ({(1, 2): 1, (1, 3): -1}, {(2, 0): 1}))),
    (({(0, 0): 1, (1, 0): 1},
      ({(1, 1): 1}, {(0, 0): 1, (1, 0): 1}), ({(1, 5): 1}, {(4, 0): 1, (5, 0): 1})),
     ({(0, 0): 1, (1, 0): 2},
      ({(0, 8): -_T, (1, 8): 2 * _T}, {(8, 0): 1}), ({(1, 3): .5}, {(2, 0): 1, (3, 0): 1})),
     ({(0, 0): 1, (1, 0): .5},
      ({(0, 8): 4 * _T, (1, 8): -2 * _T}, {(8, 0): 1}), ({(1, 7): 2}, {(6, 0): 1, (7, 0): 1})),
     ({(0, 0): 1, (1, 1): 1},
      ({(0, 0): 1, (1, 1): -1}, {(0, 0): 1, (1, 1): -1}),
      ({(0, 2): 1, (1, 3): -.5}, {(2, 0): 1, (3, 1): -2}))),
    (({(0, 1): 1, (1, 1): 1},
      ({(0, 0): 1}, {(0, 1): 1, (1, 1): 1}), ({(0, 4): 1}, {(4, 1): 1, (5, 1): 1})),
     ({(0, 1): 1, (1, 1): 2},
      ({(0, 8): -_T, (1, 8): 2 * _T}, {(8, 1): 1}), ({(0, 2): 1}, {(2, 1): 1, (3, 1): 1})),
     ({(0, 1): 1, (1, 1): .5},
      ({(0, 8): 4 * _T, (1, 8): -2 * _T}, {(8, 1): 1}), ({(0, 6): 1}, {(6, 1): 1, (7, 1): 1})),
     ({(0, 0): 1, (1, 1): .5},
      ({(0, 4): 1, (1, 5): -1}, {(4, 0): 1, (5, 1): -2}),
      ({(0, 6): 1, (1, 7): -2}, {(6, 0): 1, (7, 1): -1}))),
)
_DIAGONAL = (
    ((({(0, 1): 1, (1, 1): -1}, {(1, 0): 1, (1, 1): 1}),
      ({(0, 3): 1, (1, 3): -.5}, {(3, 0): 1, (3, 1): 2})),
     (({(0, 5): 1, (1, 5): -1}, {(5, 0): 1, (5, 1): 2}),
      ({(0, 7): 1, (1, 7): -2}, {(7, 0): 1, (7, 1): 1}))),
    ((({(0, 0): -1, (1, 0): 1}, {(0, 0): 1, (0, 1): 1}),
      ({(0, 2): -1, (1, 2): .5}, {(2, 0): 1, (2, 1): 2})),
     (({(0, 4): -.5, (1, 4): .5}, {(4, 0): 1, (4, 1): 2}),
      ({(0, 6): -.5, (1, 6): 1}, {(6, 0): 1, (6, 1): 1}))),
)
_STRASSEN = (
    ({(0, 0): 1, (1, 1): 1}, {(0, 0): 1, (1, 1): 1}, {(0, 0): 1, (1, 1): 1}),
    ({(1, 1): 1}, {(1, 0): 1, (0, 0): -1}, {(0, 0): 1, (1, 0): 1}),
    ({(0, 0): 1, (0, 1): 1}, {(1, 1): 1}, {(0, 0): -1, (0, 1): 1}),
    ({(0, 1): 1, (1, 1): -1}, {(1, 0): 1, (1, 1): 1}, {(0, 0): 1}),
    ({(1, 0): 1, (1, 1): 1}, {(0, 0): 1}, {(1, 0): 1, (1, 1): -1}),
    ({(0, 0): 1}, {(0, 1): 1, (1, 1): -1}, {(0, 1): 1, (1, 1): 1}),
    ({(1, 0): 1, (0, 0): -1}, {(0, 0): 1, (0, 1): 1}, {(1, 1): 1}),
)
_PRODUCTS = [(g, s, m) for g in range(2) for ms in (range(5), (5, 6))
             for s in range(2) for m in ms]
_WHERE = {0: (0, 0), 1: (1, 0), 2: (0, 1), 3: (1, 1),
          4: (2, 0), 5: (3, 0), 6: (2, 1), 7: (3, 1), 8: (4, None)}

_ROUNDS = "adddbcdabcddabcdabc"
_READS = "1101111111011110111"
_WRITES = "0001001100010001100"

CHUNK = 512
READ_DELAY = (0, 0)
WRITE_LEAD = 37
OUT_LAST = (2048, 1024, 512, 256, 256)


def _lincomb(terms, acc=None):
    for mag in sorted({abs(c) for c, _ in terms}, key=lambda m: (m != 1, m)):
        grp = sorted([(c, v) for c, v in terms if abs(c) == mag], key=lambda t: -t[0])
        if mag == 1 and acc is not None:
            for c, v in grp:
                acc = acc + v if c > 0 else acc - v
            continue
        sgn = 1 if grp[0][0] > 0 else -1
        s = grp[0][1]
        for c, v in grp[1:]:
            s = s + v if c * sgn > 0 else s - v
        if mag != 1:
            s = s * mag
        if acc is None:
            acc = s if sgn > 0 else -s
        else:
            acc = acc + s if sgn > 0 else acc - s
    return acc


def _prune_words(u):
    mate = lax.broadcasted_iota(jnp.int32, u.shape, 0) ^ 1
    lo = pltpu.bitcast((u << 16) & 0x7FFFFFFF, jnp.float32)
    hi = pltpu.bitcast(u & 0x7FFF0000, jnp.float32)
    big, small = jnp.maximum(lo, hi), jnp.minimum(lo, hi)
    nbig = jnp.take_along_axis(big, mate, axis=0, mode="promise_in_bounds")
    nsmall = jnp.take_along_axis(small, mate, axis=0, mode="promise_in_bounds")
    thr = jnp.maximum(jnp.minimum(big, nbig), jnp.maximum(small, nsmall))
    return u & (jnp.where(lo < thr, 0, 0xFFFF) | jnp.where(hi < thr, 0, -65536))


def _pruned_blocks(w):
    u = pltpu.bitcast(w, jnp.int32)
    return [jnp.concatenate([_prune_words(u[r:r + 8]) for r in range(k, k + KU // 2, 8)], axis=0)
            for k in range(0, u.shape[0], KU // 2)]


def _transposed(lo, hi):
    t = pltpu.bitcast(jnp.concatenate([lo, hi], axis=0), jnp.bfloat16)
    return pltpu.bitcast(t.T, jnp.int32)


def _left_operands(wt_ref, plain_ref, diag_ref):
    low = lax.broadcasted_iota(jnp.int32, (1, 128), 1) < KU

    def block(r, i, k, side):
        t, pos = _WHERE[k]
        v = wt_ref[t, pl.ds(r // 16 * 32 + 16 * i + r % 16, 8), :]
        return v if pos in (side, None) else pltpu.roll(v, KU, 1)

    def operand(r, a0, a1):
        acc = None
        for i in range(2):
            s0, s1 = ([k for k in sorted(a) if k[0] == i] for a in (a0, a1))
            for q in range(max(len(s0), len(s1))):
                c0 = a0[s0[q]] if q < len(s0) else 0
                c1 = a1[s1[q]] if q < len(s1) else 0
                if not (c0 and c1):
                    v = block(r, *s0[q], 0) if c0 else block(r, *s1[q], 1)
                elif _WHERE[s0[q][1]] == (_WHERE[s1[q][1]][0], 0):
                    v = block(r, *s0[q], 0)
                else:
                    v = jnp.where(low, block(r, *s0[q], 0), block(r, *s1[q], 1))
                v = pltpu.bitcast(v, jnp.bfloat16).astype(jnp.float32)
                if c0 == c1:
                    acc = _lincomb([(c0, v)], acc)
                else:
                    acc = _lincomb([(1, v * jnp.where(low, float(c0), float(c1)))], acc)
        return acc

    def words(v):
        return pltpu.bitcast(v.astype(jnp.bfloat16), jnp.int32)

    n = diag_ref.shape[1]
    for r in range(0, n, 8):
        for q in range(2):
            for p, (_, (a0, _), (a1, _)) in enumerate(t for rnd in _PLAIN for t in rnd):
                plain_ref[p, pl.ds(n * q + r, 8), :] = words(operand(n * q + r, a0, a1))
        for s, passes in enumerate(_DIAGONAL):
            ops = {(q, h): operand(n * q + r, a0, a1)
                   for q in range(2) for h, ((a0, _), (a1, _)) in enumerate(passes)}
            for m, (a, _, _) in enumerate(_STRASSEN):
                diag_ref[7 * s + m, pl.ds(r, 8), :] = words(
                    _lincomb([(c, ops[k]) for k, c in a.items()]))


def _kernel(x_hbm, w_hbm, b_hbm, o_hbm, xbuf, obuf, wbuf, bbuf,
            wt_ref, plain_ref, diag_ref, bias_ref, isem, fsem, osem, wsem):
    NB, NK, _, S = x_hbm.shape
    F = w_hbm.shape[1]

    def istart(b, piece, priority):
        at = (b, slice(None), pl.ds(piece[0], 8), pl.ds(*piece[1:]))
        pltpu.make_async_copy(x_hbm.at[at], xbuf.at[at], isem.at[b]).start(priority=priority)

    def iwait(b):
        pltpu.make_async_copy(x_hbm.at[b], xbuf.at[b], isem.at[b]).wait()

    def fcopy(j):
        at = (0, slice(None), slice(None), pl.ds(j * CHUNK, CHUNK))
        return pltpu.make_async_copy(x_hbm.at[at], xbuf.at[at], fsem.at[j])

    def oslot(b):
        return jnp.where(b >= OUT_SLOTS, b - OUT_SLOTS, b)

    def ostart(b, pieces):
        slot = oslot(b)
        for piece in pieces:
            at = (slice(None), pl.ds(piece[0], 8), pl.ds(*piece[1:]))
            pltpu.make_async_copy(obuf.at[(slot, *at)], o_hbm.at[(b, *at)], osem.at[b]).start()

    def owait(b):
        pltpu.make_async_copy(obuf.at[oslot(b)], o_hbm.at[b], osem.at[b]).wait()

    def wcopy(j, blocks=4):
        rows = pl.ds(pl.multiple_of(j * 4 * KU, 4 * KU), blocks * KU)
        return pltpu.make_async_copy(w_hbm.at[rows], wbuf.at[rows], wsem.at[j])

    bcopy = pltpu.make_async_copy(b_hbm, bbuf, wsem.at[3])
    bcopy.start()
    wcopy(2, 1).start()
    wcopy(0).start()
    wcopy(1).start()
    bcopy.wait()
    bias = jnp.broadcast_to(bbuf[...].reshape(1, F).astype(jnp.float32), (128, F)).T
    for i in range(2):
        bias_ref[i] = jnp.concatenate(
            [bias[k + i * KU // 2:k + (i + 1) * KU // 2] for k in range(0, F, KU)], axis=0)
    wcopy(2, 1).wait()
    last, = _pruned_blocks(wbuf[8 * KU:, :])
    wt_ref[4] = _transposed(last, last)

    @pl.loop(0, 2)
    def _(j):
        @pl.when(j == 0)
        def _():
            for c in range(S // CHUNK):
                fcopy(c).start(priority=int(c >= 2))

        wcopy(j).wait()
        u = _pruned_blocks(wbuf[pl.ds(pl.multiple_of(j * 4 * KU, 4 * KU), 4 * KU), :])
        for e in range(2):
            wt_ref[2 * j + e] = _transposed(u[e], u[e + 2])

    _left_operands(wt_ref, plain_ref, diag_ref)

    def xblock(i, o, k, j):
        return xbuf[i, k, :, pl.ds(o + 128 * j, 128)]

    def right(i, o, b0, b1):
        return jnp.concatenate(
            [_lincomb([(c, xblock(i, o, *kj).astype(jnp.float32)) for kj, c in t.items()])
             for t in (b0, b1)], axis=0)

    def matmul(words, rhs):
        return jnp.dot(pltpu.bitcast(words, jnp.bfloat16), rhs.astype(jnp.bfloat16),
                       preferred_element_type=jnp.float32)

    def plain_round(i, slot, o, n, acc):
        ms = []
        for q, (_, (_, b0), (_, b1)) in enumerate(_PLAIN[n]):
            if len(b0) == len(b1) == 1:
                rhs = jnp.concatenate([xblock(i, o, *min(b0)), xblock(i, o, *min(b1))], axis=0)
            else:
                rhs = right(i, o, b0, b1)
            ms.append(matmul(plain_ref[4 * n + q], rhs))
        for c in ((0, 0), (0, 1), (1, 0), (1, 1)):
            terms = [(t[0][c], v) for t, v in zip(_PLAIN[n], ms) if c in t[0]]
            if not terms:
                continue
            acc[c] = _lincomb(terms, acc[c] if c in acc else bias_ref[c[0]])
            if not any(c in t[0] for rnd in _PLAIN[n + 1:] for t in rnd):
                obuf[slot, :, pl.ds(KU // 2 * c[0], KU // 2), pl.ds(o + 128 * c[1], 128)] = (
                    acc[c].astype(obuf.dtype).reshape(NK, KU // 2, 128))

    def diagonal_round(i, o, products, accs, rights):
        ms = []
        for g, s, m in products:
            for h, p in _STRASSEN[m][1]:
                if (g, s, h, p) not in rights:
                    (_, b0), (_, b1) = _DIAGONAL[s][h]
                    rights[g, s, h, p] = right(i, o + PAIR * (2 * g + p), b0, b1)
            rhs = _lincomb([(c, rights[g, s, h, p]) for (h, p), c in _STRASSEN[m][1].items()])
            ms.append(matmul(diag_ref[7 * s + m], rhs))
        n = F // 4
        for g, s in sorted({t[:2] for t in products}):
            for p in range(2):
                terms = [[(_STRASSEN[t[2]][2][q, p], v) for t, v in zip(products, ms)
                          if t[:2] == (g, s) and (q, p) in _STRASSEN[t[2]][2]] for q in range(2)]
                if any(terms):
                    acc = accs[2 * g + p]
                    prev = acc[s, s] if (s, s) in acc else bias_ref[s]
                    acc[s, s] = jnp.concatenate(
                        [_lincomb(terms[q], prev[n * q:n * q + n]) for q in range(2)], axis=0)

    reads = ([(0, o, 128) for o in range(0, S, 128)],
             [(r, o, CHUNK) for r in range(8, KU, 8) for o in range(0, S, CHUNK)])
    writes = [(r, o, CHUNK) for r in range(0, KU, 8) for o in range(0, S, CHUNK)]
    last_writes = {}
    for j, n in enumerate(OUT_LAST):
        o = sum(OUT_LAST[:j])
        last_writes[o + n] = [(r, c, min(CHUNK, n)) for r in range(0, KU, 8)
                              for c in range(o, o + n, CHUNK)]
    read_steps = S // (4 * PAIR) * _READS.count("1")
    write_steps = S // (4 * PAIR) * _WRITES.count("1")

    def share(pieces, step, steps):
        return range(step * 2 * len(pieces) // steps, (step + 1) * 2 * len(pieces) // steps)

    @pl.loop(0, NB)
    def _(i):
        @pl.when(i > 0)
        def _():
            iwait(i)

        @pl.when(i >= OUT_SLOTS)
        def _():
            owait(i - OUT_SLOTS)

        slot = oslot(i)
        ready = rstep = wstep = 0
        pending = []
        for o in range(0, S, 4 * PAIR):
            accs = [{} for _ in range(4)]
            rights = {}
            for t, kind in enumerate(_ROUNDS):
                k = _ROUNDS[:t].count(kind)
                products = _PRODUCTS[4 * k:4 * k + 4]
                pairs = (2 * products[-1][0] + 2 if kind == "d"
                         else k + 3 if kind == "c" else k + 1)
                while ready * CHUNK < min(o + PAIR * pairs, S):
                    @pl.when(i == 0)
                    def _():
                        fcopy(ready).wait()
                    ready += 1

                if kind == "d":
                    diagonal_round(i, o, products, accs, rights)
                else:
                    plain_round(i, slot, o + PAIR * k, "abc".index(kind), accs[k])

                if _READS[t] == "1":
                    for priority, pieces in enumerate(reads):
                        for q in share(pieces, rstep, read_steps):
                            db, q = divmod(q - READ_DELAY[priority], len(pieces))
                            b = 2 * i + 1 + db

                            @pl.when((b >= 1) & (b < NB))
                            def _():
                                istart(b, pieces[q], priority)
                    rstep += 1
                if _WRITES[t] == "1":
                    qs = [divmod(q + WRITE_LEAD, len(writes))
                          for q in share(writes, wstep, write_steps)]
                    for db in sorted({d for d, _ in qs}):
                        b = 2 * i - NB + db

                        @pl.when((b >= 0) & (b < NB - 1))
                        def _():
                            ostart(b, [writes[q] for d, q in qs if d == db])
                    wstep += 1
                    if pending:
                        @pl.when(i == NB - 1)
                        def _():
                            ostart(NB - 1, pending[:16])
                        del pending[:16]
                if kind == "c":
                    pending += last_writes.get(o + PAIR * (k + 1), [])
        last_writes[S] = pending

    ostart(NB - 1, last_writes[S])
    for b in range(NB - OUT_SLOTS, NB):
        owait(b)


@jax.jit
def pallas_standalone__structured_sparse_n_m__ragged_kernel(
    x: jax.Array,
    w: jax.Array,
    b: jax.Array,
):
    B, S, D = x.shape
    F = w.shape[1]
    xt = jnp.transpose(x, (0, 2, 1)).reshape(B, D // KU, KU, S)
    out = pl.pallas_call(
        _kernel,
        in_specs=[pl.BlockSpec(memory_space=pl.ANY)] * 3,
        out_specs=pl.BlockSpec(memory_space=pl.ANY),
        out_shape=jax.ShapeDtypeStruct((B, F // KU, KU, S), x.dtype),
        scratch_shapes=[
            pltpu.VMEM((B, D // KU, KU, S), x.dtype),
            pltpu.VMEM((OUT_SLOTS, F // KU, KU, S), x.dtype),
            pltpu.VMEM((D, F), w.dtype),
            pltpu.VMEM((F,), b.dtype),
            pltpu.VMEM((5, F // 2, 128), jnp.int32),
            pltpu.VMEM((12, F // 4, 128), jnp.int32),
            pltpu.VMEM((14, F // 8, 128), jnp.int32),
            pltpu.VMEM((2, F // 2, 128), jnp.float32),
            pltpu.SemaphoreType.DMA((B,)),
            pltpu.SemaphoreType.DMA((S // CHUNK,)),
            pltpu.SemaphoreType.DMA((B,)),
            pltpu.SemaphoreType.DMA((4,)),
        ],
        compiler_params=pltpu.CompilerParams(
            vmem_limit_bytes=120 * 1024 * 1024,
            disable_bounds_checks=True,
            disable_semaphore_checks=True,
            flags={"XLA_TPU_RESCHEDULE_DMA_DONES": True},
        ),
    )(xt, w, b)
    return jnp.transpose(out.reshape(B, F, S), (0, 2, 1))
```

```python
import jax
import jax.numpy as jnp
from jax import lax
import jax.experimental.pallas as pl
import jax.experimental.pallas.tpu as pltpu

KU = 64
PAIR = 256
OUT_SLOTS = 9

_T = 1.0 / 3.0
_PLAIN = (
    (({(0, 0): 1, (0, 1): -1},
      ({(0, 0): 1, (0, 1): -1}, {(1, 1): 1}), ({(0, 6): 1, (0, 7): -1}, {(7, 1): 1})),
     ({(0, 0): 1, (0, 1): -.5},
      ({(0, 4): 2, (0, 5): -2}, {(5, 1): 1}), ({(0, 2): 2, (0, 3): -2}, {(3, 1): 1})),
     ({(1, 0): 1, (1, 1): -1},
      ({(1, 0): 1, (1, 1): -1}, {(0, 0): 1}), ({(1, 6): 1, (1, 7): -1}, {(6, 0): 1})),
     ({(1, 0): 1, (1, 1): -.5},
      ({(1, 4): 1, (1, 5): -1}, {(4, 0): 1}), ({(1, 2): 1, (1, 3): -1}, {(2, 0): 1}))),
    (({(0, 0): 1, (1, 0): 1},
      ({(1, 1): 1}, {(0, 0): 1, (1, 0): 1}), ({(1, 5): 1}, {(4, 0): 1, (5, 0): 1})),
     ({(0, 0): 1, (1, 0): 2},
      ({(0, 8): -_T, (1, 8): 2 * _T}, {(8, 0): 1}), ({(1, 3): .5}, {(2, 0): 1, (3, 0): 1})),
     ({(0, 0): 1, (1, 0): .5},
      ({(0, 8): 4 * _T, (1, 8): -2 * _T}, {(8, 0): 1}), ({(1, 7): 2}, {(6, 0): 1, (7, 0): 1})),
     ({(0, 0): 1, (1, 1): 1},
      ({(0, 0): 1, (1, 1): -1}, {(0, 0): 1, (1, 1): -1}),
      ({(0, 2): 1, (1, 3): -.5}, {(2, 0): 1, (3, 1): -2}))),
    (({(0, 1): 1, (1, 1): 1},
      ({(0, 0): 1}, {(0, 1): 1, (1, 1): 1}), ({(0, 4): 1}, {(4, 1): 1, (5, 1): 1})),
     ({(0, 1): 1, (1, 1): 2},
      ({(0, 8): -_T, (1, 8): 2 * _T}, {(8, 1): 1}), ({(0, 2): 1}, {(2, 1): 1, (3, 1): 1})),
     ({(0, 1): 1, (1, 1): .5},
      ({(0, 8): 4 * _T, (1, 8): -2 * _T}, {(8, 1): 1}), ({(0, 6): 1}, {(6, 1): 1, (7, 1): 1})),
     ({(0, 0): 1, (1, 1): .5},
      ({(0, 4): 1, (1, 5): -1}, {(4, 0): 1, (5, 1): -2}),
      ({(0, 6): 1, (1, 7): -2}, {(6, 0): 1, (7, 1): -1}))),
)
_DIAGONAL = (
    ((({(0, 1): 1, (1, 1): -1}, {(1, 0): 1, (1, 1): 1}),
      ({(0, 3): 1, (1, 3): -.5}, {(3, 0): 1, (3, 1): 2})),
     (({(0, 5): 1, (1, 5): -1}, {(5, 0): 1, (5, 1): 2}),
      ({(0, 7): 1, (1, 7): -2}, {(7, 0): 1, (7, 1): 1}))),
    ((({(0, 0): -1, (1, 0): 1}, {(0, 0): 1, (0, 1): 1}),
      ({(0, 2): -1, (1, 2): .5}, {(2, 0): 1, (2, 1): 2})),
     (({(0, 4): -.5, (1, 4): .5}, {(4, 0): 1, (4, 1): 2}),
      ({(0, 6): -.5, (1, 6): 1}, {(6, 0): 1, (6, 1): 1}))),
)
_STRASSEN = (
    ({(0, 0): 1, (1, 1): 1}, {(0, 0): 1, (1, 1): 1}, {(0, 0): 1, (1, 1): 1}),
    ({(1, 1): 1}, {(1, 0): 1, (0, 0): -1}, {(0, 0): 1, (1, 0): 1}),
    ({(0, 0): 1, (0, 1): 1}, {(1, 1): 1}, {(0, 0): -1, (0, 1): 1}),
    ({(0, 1): 1, (1, 1): -1}, {(1, 0): 1, (1, 1): 1}, {(0, 0): 1}),
    ({(1, 0): 1, (1, 1): 1}, {(0, 0): 1}, {(1, 0): 1, (1, 1): -1}),
    ({(0, 0): 1}, {(0, 1): 1, (1, 1): -1}, {(0, 1): 1, (1, 1): 1}),
    ({(1, 0): 1, (0, 0): -1}, {(0, 0): 1, (0, 1): 1}, {(1, 1): 1}),
)
_PRODUCTS = [(g, s, m) for g in range(2) for ms in (range(5), (5, 6))
             for s in range(2) for m in ms]
_WHERE = {0: (0, 0), 1: (1, 0), 2: (0, 1), 3: (1, 1),
          4: (2, 0), 5: (3, 0), 6: (2, 1), 7: (3, 1), 8: (4, None)}

_ROUNDS = "adddbcdabcddabcdabc"
_READS = "1101111111011110111"
_WRITES = "0001001100010001100"

CHUNK = 512
READ_DELAY = (0, 0)
WRITE_LEAD = 37
OUT_LAST = ((2048, 2048), (2048, 1024, 512, 256, 256))


def _lincomb(terms, acc=None):
    for mag in sorted({abs(c) for c, _ in terms}, key=lambda m: (m != 1, m)):
        grp = sorted([(c, v) for c, v in terms if abs(c) == mag], key=lambda t: -t[0])
        if mag == 1 and acc is not None:
            for c, v in grp:
                acc = acc + v if c > 0 else acc - v
            continue
        sgn = 1 if grp[0][0] > 0 else -1
        s = grp[0][1]
        for c, v in grp[1:]:
            s = s + v if c * sgn > 0 else s - v
        if mag != 1:
            s = s * mag
        if acc is None:
            acc = s if sgn > 0 else -s
        else:
            acc = acc + s if sgn > 0 else acc - s
    return acc


def _prune_words(u):
    mate = lax.broadcasted_iota(jnp.int32, u.shape, 0) ^ 1
    lo = pltpu.bitcast((u << 16) & 0x7FFFFFFF, jnp.float32)
    hi = pltpu.bitcast(u & 0x7FFF0000, jnp.float32)
    big, small = jnp.maximum(lo, hi), jnp.minimum(lo, hi)
    nbig = jnp.take_along_axis(big, mate, axis=0, mode="promise_in_bounds")
    nsmall = jnp.take_along_axis(small, mate, axis=0, mode="promise_in_bounds")
    thr = jnp.maximum(jnp.minimum(big, nbig), jnp.maximum(small, nsmall))
    return u & (jnp.where(lo < thr, 0, 0xFFFF) | jnp.where(hi < thr, 0, -65536))


def _pruned_blocks(w):
    u = pltpu.bitcast(w, jnp.int32)
    return [jnp.concatenate([_prune_words(u[r:r + 8]) for r in range(k, k + KU // 2, 8)], axis=0)
            for k in range(0, u.shape[0], KU // 2)]


def _transposed(lo, hi):
    t = pltpu.bitcast(jnp.concatenate([lo, hi], axis=0), jnp.bfloat16)
    return pltpu.bitcast(t.T, jnp.int32)


def _left_operands(wt_ref, plain_ref, diag_ref):
    low = lax.broadcasted_iota(jnp.int32, (1, 128), 1) < KU

    def block(r, i, k, side):
        t, pos = _WHERE[k]
        v = wt_ref[t, pl.ds(r // 16 * 32 + 16 * i + r % 16, 8), :]
        return v if pos in (side, None) else pltpu.roll(v, KU, 1)

    def operand(r, a0, a1):
        acc = None
        for i in range(2):
            s0, s1 = ([k for k in sorted(a) if k[0] == i] for a in (a0, a1))
            for q in range(max(len(s0), len(s1))):
                c0 = a0[s0[q]] if q < len(s0) else 0
                c1 = a1[s1[q]] if q < len(s1) else 0
                if not (c0 and c1):
                    v = block(r, *s0[q], 0) if c0 else block(r, *s1[q], 1)
                elif _WHERE[s0[q][1]] == (_WHERE[s1[q][1]][0], 0):
                    v = block(r, *s0[q], 0)
                else:
                    v = jnp.where(low, block(r, *s0[q], 0), block(r, *s1[q], 1))
                v = pltpu.bitcast(v, jnp.bfloat16).astype(jnp.float32)
                if c0 == c1:
                    acc = _lincomb([(c0, v)], acc)
                else:
                    acc = _lincomb([(1, v * jnp.where(low, float(c0), float(c1)))], acc)
        return acc

    def words(v):
        return pltpu.bitcast(v.astype(jnp.bfloat16), jnp.int32)

    n = diag_ref.shape[1]
    for r in range(0, n, 8):
        for q in range(2):
            for p, (_, (a0, _), (a1, _)) in enumerate(t for rnd in _PLAIN for t in rnd):
                plain_ref[p, pl.ds(n * q + r, 8), :] = words(operand(n * q + r, a0, a1))
        for s, passes in enumerate(_DIAGONAL):
            ops = {(q, h): operand(n * q + r, a0, a1)
                   for q in range(2) for h, ((a0, _), (a1, _)) in enumerate(passes)}
            for m, (a, _, _) in enumerate(_STRASSEN):
                diag_ref[7 * s + m, pl.ds(r, 8), :] = words(
                    _lincomb([(c, ops[k]) for k, c in a.items()]))


def _kernel(x_hbm, w_hbm, b_hbm, o_hbm, xbuf, obuf, wbuf, bbuf,
            wt_ref, plain_ref, diag_ref, bias_ref, isem, fsem, osem, wsem):
    NB, NK, _, S = x_hbm.shape
    F = w_hbm.shape[1]

    def istart(b, piece, priority):
        at = (b, slice(None), pl.ds(piece[0], 8), pl.ds(*piece[1:]))
        pltpu.make_async_copy(x_hbm.at[at], xbuf.at[at], isem.at[b]).start(priority=priority)

    def iwait(b):
        pltpu.make_async_copy(x_hbm.at[b], xbuf.at[b], isem.at[b]).wait()

    def fcopy(j):
        at = (0, slice(None), slice(None), pl.ds(j * CHUNK, CHUNK))
        return pltpu.make_async_copy(x_hbm.at[at], xbuf.at[at], fsem.at[j])

    def oslot(b):
        return jnp.where(b >= OUT_SLOTS, b - OUT_SLOTS, b)

    def ostart(b, pieces):
        slot = oslot(b)
        for piece in pieces:
            at = (slice(None), pl.ds(piece[0], 8), pl.ds(*piece[1:]))
            pltpu.make_async_copy(obuf.at[(slot, *at)], o_hbm.at[(b, *at)], osem.at[b]).start()

    def owait(b):
        pltpu.make_async_copy(obuf.at[oslot(b)], o_hbm.at[b], osem.at[b]).wait()

    def wcopy(j, blocks=4):
        rows = pl.ds(pl.multiple_of(j * 4 * KU, 4 * KU), blocks * KU)
        return pltpu.make_async_copy(w_hbm.at[rows], wbuf.at[rows], wsem.at[j])

    bcopy = pltpu.make_async_copy(b_hbm, bbuf, wsem.at[3])
    bcopy.start()
    wcopy(2, 1).start()
    wcopy(0).start()
    wcopy(1).start()
    bcopy.wait()
    bias = jnp.broadcast_to(bbuf[...].reshape(1, F).astype(jnp.float32), (128, F)).T
    for i in range(2):
        bias_ref[i] = jnp.concatenate(
            [bias[k + i * KU // 2:k + (i + 1) * KU // 2] for k in range(0, F, KU)], axis=0)
    wcopy(2, 1).wait()
    ninth, = _pruned_blocks(wbuf[8 * KU:, :])
    wt_ref[4] = _transposed(ninth, ninth)

    @pl.loop(0, 2)
    def _(j):
        @pl.when(j == 0)
        def _():
            for c in range(S // CHUNK):
                fcopy(c).start(priority=int(c >= 2))

        wcopy(j).wait()
        u = _pruned_blocks(wbuf[pl.ds(pl.multiple_of(j * 4 * KU, 4 * KU), 4 * KU), :])
        for e in range(2):
            wt_ref[2 * j + e] = _transposed(u[e], u[e + 2])

    _left_operands(wt_ref, plain_ref, diag_ref)

    def xblock(i, o, k, j):
        return xbuf[i, k, :, pl.ds(o + 128 * j, 128)]

    def right(i, o, b0, b1):
        return jnp.concatenate(
            [_lincomb([(c, xblock(i, o, *kj).astype(jnp.float32)) for kj, c in t.items()])
             for t in (b0, b1)], axis=0)

    def matmul(words, rhs):
        return jnp.dot(pltpu.bitcast(words, jnp.bfloat16), rhs.astype(jnp.bfloat16),
                       preferred_element_type=jnp.float32)

    def plain_round(i, slot, o, n, acc):
        ms = []
        for q, (_, (_, b0), (_, b1)) in enumerate(_PLAIN[n]):
            if len(b0) == len(b1) == 1:
                rhs = jnp.concatenate([xblock(i, o, *min(b0)), xblock(i, o, *min(b1))], axis=0)
            else:
                rhs = right(i, o, b0, b1)
            ms.append(matmul(plain_ref[4 * n + q], rhs))
        for c in ((0, 0), (0, 1), (1, 0), (1, 1)):
            terms = [(t[0][c], v) for t, v in zip(_PLAIN[n], ms) if c in t[0]]
            if not terms:
                continue
            acc[c] = _lincomb(terms, acc[c] if c in acc else bias_ref[c[0]])
            if not any(c in t[0] for rnd in _PLAIN[n + 1:] for t in rnd):
                obuf[slot, :, pl.ds(KU // 2 * c[0], KU // 2), pl.ds(o + 128 * c[1], 128)] = (
                    acc[c].astype(obuf.dtype).reshape(NK, KU // 2, 128))

    def diagonal_round(i, o, products, accs, rights):
        ms = []
        for g, s, m in products:
            for h, p in _STRASSEN[m][1]:
                if (g, s, h, p) not in rights:
                    (_, b0), (_, b1) = _DIAGONAL[s][h]
                    rights[g, s, h, p] = right(i, o + PAIR * (2 * g + p), b0, b1)
            rhs = _lincomb([(c, rights[g, s, h, p]) for (h, p), c in _STRASSEN[m][1].items()])
            ms.append(matmul(diag_ref[7 * s + m], rhs))
        n = F // 4
        for g, s in sorted({t[:2] for t in products}):
            for p in range(2):
                terms = [[(_STRASSEN[t[2]][2][q, p], v) for t, v in zip(products, ms)
                          if t[:2] == (g, s) and (q, p) in _STRASSEN[t[2]][2]] for q in range(2)]
                if any(terms):
                    acc = accs[2 * g + p]
                    prev = acc[s, s] if (s, s) in acc else bias_ref[s]
                    acc[s, s] = jnp.concatenate(
                        [_lincomb(terms[q], prev[n * q:n * q + n]) for q in range(2)], axis=0)

    reads = ([(0, o, 128) for o in range(0, S, 128)],
             [(r, o, CHUNK) for r in range(8, KU, 8) for o in range(0, S, CHUNK)])
    writes = [(r, o, CHUNK) for r in range(0, KU, 8) for o in range(0, S, CHUNK)]
    steady = NB - len(OUT_LAST)
    assert WRITE_LEAD <= len(writes) and len(OUT_LAST) >= 2
    last = [(steady + e, sum(sizes[:j + 1]), (r, c, min(CHUNK, n)))
            for e, sizes in enumerate(OUT_LAST) for j, n in enumerate(sizes)
            for r in range(0, KU, 8)
            for c in range(sum(sizes[:j]), sum(sizes[:j + 1]), CHUNK)]
    read_steps = S // (4 * PAIR) * _READS.count("1")
    write_steps = S // (4 * PAIR) * _WRITES.count("1")

    def share(pieces, step, steps):
        return range(step * 2 * len(pieces) // steps, (step + 1) * 2 * len(pieces) // steps)

    last_writes = {}
    position = steady * len(writes)
    for i in range(steady, NB):
        done = wstep = 0
        for t, kind in enumerate(S // (4 * PAIR) * _ROUNDS):
            done += PAIR * (kind == "c")
            if _WRITES[t % len(_ROUNDS)] == "1":
                due = ((2 * i - NB) * len(writes) + WRITE_LEAD
                       + share(writes, wstep, write_steps).stop)
                while last and position < due and last[0][:2] <= (i, done):
                    b, _, piece = last.pop(0)
                    last_writes.setdefault((i, wstep), []).append((b, piece))
                    position += piece[2] / CHUNK
                wstep += 1

    @pl.loop(0, NB)
    def _(i):
        @pl.when(i > 0)
        def _():
            iwait(i)

        @pl.when(i >= OUT_SLOTS)
        def _():
            owait(i - OUT_SLOTS)

        slot = oslot(i)
        ready = rstep = wstep = 0
        for o in range(0, S, 4 * PAIR):
            accs = [{} for _ in range(4)]
            rights = {}
            for t, kind in enumerate(_ROUNDS):
                k = _ROUNDS[:t].count(kind)
                products = _PRODUCTS[4 * k:4 * k + 4]
                pairs = (2 * products[-1][0] + 2 if kind == "d"
                         else k + 3 if kind == "c" else k + 1)
                while ready * CHUNK < min(o + PAIR * pairs, S):
                    @pl.when(i == 0)
                    def _():
                        fcopy(ready).wait()
                    ready += 1

                if kind == "d":
                    diagonal_round(i, o, products, accs, rights)
                else:
                    plain_round(i, slot, o + PAIR * k, "abc".index(kind), accs[k])

                if _READS[t] == "1":
                    for priority, pieces in enumerate(reads):
                        for q in share(pieces, rstep, read_steps):
                            db, q = divmod(q - READ_DELAY[priority], len(pieces))
                            b = 2 * i + 1 + db

                            @pl.when((b >= 1) & (b < NB))
                            def _():
                                istart(b, pieces[q], priority)
                    rstep += 1
                if _WRITES[t] == "1":
                    qs = [divmod(q + WRITE_LEAD, len(writes))
                          for q in share(writes, wstep, write_steps)]
                    for db in sorted({d for d, _ in qs}):
                        b = 2 * i - NB + db

                        @pl.when((b >= 0) & (b < steady))
                        def _():
                            ostart(b, [writes[q] for d, q in qs if d == db])
                    for it in range(steady, NB):
                        if (it, wstep) in last_writes:
                            @pl.when(i == it)
                            def _():
                                for b, piece in last_writes[it, wstep]:
                                    ostart(b, [piece])
                    wstep += 1

    for b, _, piece in last:
        ostart(b, [piece])
    for b in range(NB - OUT_SLOTS, NB):
        owait(b)


@jax.jit
def pallas_standalone__structured_sparse_n_m__ragged_kernel(
    x: jax.Array,
    w: jax.Array,
    b: jax.Array,
):
    B, S, D = x.shape
    F = w.shape[1]
    xt = jnp.transpose(x, (0, 2, 1)).reshape(B, D // KU, KU, S)
    out = pl.pallas_call(
        _kernel,
        in_specs=[pl.BlockSpec(memory_space=pl.ANY)] * 3,
        out_specs=pl.BlockSpec(memory_space=pl.ANY),
        out_shape=jax.ShapeDtypeStruct((B, F // KU, KU, S), x.dtype),
        scratch_shapes=[
            pltpu.VMEM((B, D // KU, KU, S), x.dtype),
            pltpu.VMEM((OUT_SLOTS, F // KU, KU, S), x.dtype),
            pltpu.VMEM((D, F), w.dtype),
            pltpu.VMEM((F,), b.dtype),
            pltpu.VMEM((5, F // 2, 128), jnp.int32),
            pltpu.VMEM((12, F // 4, 128), jnp.int32),
            pltpu.VMEM((14, F // 8, 128), jnp.int32),
            pltpu.VMEM((2, F // 2, 128), jnp.float32),
            pltpu.SemaphoreType.DMA((B,)),
            pltpu.SemaphoreType.DMA((S // CHUNK,)),
            pltpu.SemaphoreType.DMA((B,)),
            pltpu.SemaphoreType.DMA((4,)),
        ],
        compiler_params=pltpu.CompilerParams(
            vmem_limit_bytes=120 * 1024 * 1024,
            disable_bounds_checks=True,
            disable_semaphore_checks=True,
            flags={"XLA_TPU_RESCHEDULE_DMA_DONES": True},
        ),
    )(xt, w, b)
    return jnp.transpose(out.reshape(B, F, S), (0, 2, 1))
```

```python
import jax
import jax.numpy as jnp
from jax import lax
import jax.experimental.pallas as pl
import jax.experimental.pallas.tpu as pltpu

KU = 64
PAIR = 256
OUT_SLOTS = 9

_T = 1.0 / 3.0
_PLAIN = (
    (({(0, 0): 1, (0, 1): -1},
      ({(0, 0): 1, (0, 1): -1}, {(1, 1): 1}), ({(0, 6): 1, (0, 7): -1}, {(7, 1): 1})),
     ({(0, 0): 1, (0, 1): -.5},
      ({(0, 4): 2, (0, 5): -2}, {(5, 1): 1}), ({(0, 2): 2, (0, 3): -2}, {(3, 1): 1})),
     ({(1, 0): 1, (1, 1): -1},
      ({(1, 0): 1, (1, 1): -1}, {(0, 0): 1}), ({(1, 6): 1, (1, 7): -1}, {(6, 0): 1})),
     ({(1, 0): 1, (1, 1): -.5},
      ({(1, 4): 1, (1, 5): -1}, {(4, 0): 1}), ({(1, 2): 1, (1, 3): -1}, {(2, 0): 1}))),
    (({(0, 0): 1, (1, 0): 1},
      ({(1, 1): 1}, {(0, 0): 1, (1, 0): 1}), ({(1, 5): 1}, {(4, 0): 1, (5, 0): 1})),
     ({(0, 0): 1, (1, 0): 2},
      ({(0, 8): -_T, (1, 8): 2 * _T}, {(8, 0): 1}), ({(1, 3): .5}, {(2, 0): 1, (3, 0): 1})),
     ({(0, 0): 1, (1, 0): .5},
      ({(0, 8): 4 * _T, (1, 8): -2 * _T}, {(8, 0): 1}), ({(1, 7): 2}, {(6, 0): 1, (7, 0): 1})),
     ({(0, 0): 1, (1, 1): 1},
      ({(0, 0): 1, (1, 1): -1}, {(0, 0): 1, (1, 1): -1}),
      ({(0, 2): 1, (1, 3): -.5}, {(2, 0): 1, (3, 1): -2}))),
    (({(0, 1): 1, (1, 1): 1},
      ({(0, 0): 1}, {(0, 1): 1, (1, 1): 1}), ({(0, 4): 1}, {(4, 1): 1, (5, 1): 1})),
     ({(0, 1): 1, (1, 1): 2},
      ({(0, 8): -_T, (1, 8): 2 * _T}, {(8, 1): 1}), ({(0, 2): 1}, {(2, 1): 1, (3, 1): 1})),
     ({(0, 1): 1, (1, 1): .5},
      ({(0, 8): 4 * _T, (1, 8): -2 * _T}, {(8, 1): 1}), ({(0, 6): 1}, {(6, 1): 1, (7, 1): 1})),
     ({(0, 0): 1, (1, 1): .5},
      ({(0, 4): 1, (1, 5): -1}, {(4, 0): 1, (5, 1): -2}),
      ({(0, 6): 1, (1, 7): -2}, {(6, 0): 1, (7, 1): -1}))),
)
_DIAGONAL = (
    ((({(0, 1): 1, (1, 1): -1}, {(1, 0): 1, (1, 1): 1}),
      ({(0, 3): 1, (1, 3): -.5}, {(3, 0): 1, (3, 1): 2})),
     (({(0, 5): 1, (1, 5): -1}, {(5, 0): 1, (5, 1): 2}),
      ({(0, 7): 1, (1, 7): -2}, {(7, 0): 1, (7, 1): 1}))),
    ((({(0, 0): -1, (1, 0): 1}, {(0, 0): 1, (0, 1): 1}),
      ({(0, 2): -1, (1, 2): .5}, {(2, 0): 1, (2, 1): 2})),
     (({(0, 4): -.5, (1, 4): .5}, {(4, 0): 1, (4, 1): 2}),
      ({(0, 6): -.5, (1, 6): 1}, {(6, 0): 1, (6, 1): 1}))),
)
_STRASSEN = (
    ({(0, 0): 1, (1, 1): 1}, {(0, 0): 1, (1, 1): 1}, {(0, 0): 1, (1, 1): 1}),
    ({(1, 1): 1}, {(1, 0): 1, (0, 0): -1}, {(0, 0): 1, (1, 0): 1}),
    ({(0, 0): 1, (0, 1): 1}, {(1, 1): 1}, {(0, 0): -1, (0, 1): 1}),
    ({(0, 1): 1, (1, 1): -1}, {(1, 0): 1, (1, 1): 1}, {(0, 0): 1}),
    ({(1, 0): 1, (1, 1): 1}, {(0, 0): 1}, {(1, 0): 1, (1, 1): -1}),
    ({(0, 0): 1}, {(0, 1): 1, (1, 1): -1}, {(0, 1): 1, (1, 1): 1}),
    ({(1, 0): 1, (0, 0): -1}, {(0, 0): 1, (0, 1): 1}, {(1, 1): 1}),
)
_PRODUCTS = [(g, s, m) for g in range(2) for ms in (range(5), (5, 6))
             for s in range(2) for m in ms]
_WHERE = {0: (0, 0), 1: (1, 0), 2: (0, 1), 3: (1, 1),
          4: (2, 0), 5: (3, 0), 6: (2, 1), 7: (3, 1), 8: (4, None)}

_ROUNDS = "adddbcdabcddabcdabc"
_READS = "1101111111011110111"
_WRITES = "0001001100010001100"

CHUNK = 512
READ_DELAY = (0, 0)
WRITE_LEAD = 37
OUT_LAST = ((2048, 2048), (2048, 1024, 512, 256, 256))


def _lincomb(terms, acc=None):
    for mag in sorted({abs(c) for c, _ in terms}, key=lambda m: (m != 1, m)):
        grp = sorted([(c, v) for c, v in terms if abs(c) == mag], key=lambda t: -t[0])
        if mag == 1 and acc is not None:
            for c, v in grp:
                acc = acc + v if c > 0 else acc - v
            continue
        sgn = 1 if grp[0][0] > 0 else -1
        s = grp[0][1]
        for c, v in grp[1:]:
            s = s + v if c * sgn > 0 else s - v
        if mag != 1:
            s = s * mag
        if acc is None:
            acc = s if sgn > 0 else -s
        else:
            acc = acc + s if sgn > 0 else acc - s
    return acc


def _prune_words(u):
    mate = lax.broadcasted_iota(jnp.int32, u.shape, 0) ^ 1
    lo = pltpu.bitcast((u << 16) & 0x7FFFFFFF, jnp.float32)
    hi = pltpu.bitcast(u & 0x7FFF0000, jnp.float32)
    big, small = jnp.maximum(lo, hi), jnp.minimum(lo, hi)
    nbig = jnp.take_along_axis(big, mate, axis=0, mode="promise_in_bounds")
    nsmall = jnp.take_along_axis(small, mate, axis=0, mode="promise_in_bounds")
    thr = jnp.maximum(jnp.minimum(big, nbig), jnp.maximum(small, nsmall))
    return u & (jnp.where(lo < thr, 0, 0xFFFF) | jnp.where(hi < thr, 0, -65536))


def _pruned_blocks(w):
    u = pltpu.bitcast(w, jnp.int32)
    return [jnp.concatenate([_prune_words(u[r:r + 8]) for r in range(k, k + KU // 2, 8)], axis=0)
            for k in range(0, u.shape[0], KU // 2)]


def _transposed(lo, hi):
    t = pltpu.bitcast(jnp.concatenate([lo, hi], axis=0), jnp.bfloat16)
    return pltpu.bitcast(t.T, jnp.int32)


def _left_operands(wt_ref, plain_ref, diag_ref):
    low = lax.broadcasted_iota(jnp.int32, (1, 128), 1) < KU

    def block(r, i, k, side):
        t, pos = _WHERE[k]
        v = wt_ref[t, pl.ds(r // 16 * 32 + 16 * i + r % 16, 8), :]
        return v if pos in (side, None) else pltpu.roll(v, KU, 1)

    def operand(r, a0, a1):
        acc = None
        for i in range(2):
            s0, s1 = ([k for k in sorted(a) if k[0] == i] for a in (a0, a1))
            for q in range(max(len(s0), len(s1))):
                c0 = a0[s0[q]] if q < len(s0) else 0
                c1 = a1[s1[q]] if q < len(s1) else 0
                if not (c0 and c1):
                    v = block(r, *s0[q], 0) if c0 else block(r, *s1[q], 1)
                elif _WHERE[s0[q][1]] == (_WHERE[s1[q][1]][0], 0):
                    v = block(r, *s0[q], 0)
                else:
                    v = jnp.where(low, block(r, *s0[q], 0), block(r, *s1[q], 1))
                v = pltpu.bitcast(v, jnp.bfloat16).astype(jnp.float32)
                if c0 == c1:
                    acc = _lincomb([(c0, v)], acc)
                else:
                    acc = _lincomb([(1, v * jnp.where(low, float(c0), float(c1)))], acc)
        return acc

    def words(v):
        return pltpu.bitcast(v.astype(jnp.bfloat16), jnp.int32)

    n = diag_ref.shape[1]
    for r in range(0, n, 8):
        for q in range(2):
            for p, (_, (a0, _), (a1, _)) in enumerate(t for rnd in _PLAIN for t in rnd):
                plain_ref[p, pl.ds(n * q + r, 8), :] = words(operand(n * q + r, a0, a1))
        for s, passes in enumerate(_DIAGONAL):
            ops = {(q, h): operand(n * q + r, a0, a1)
                   for q in range(2) for h, ((a0, _), (a1, _)) in enumerate(passes)}
            for m, (a, _, _) in enumerate(_STRASSEN):
                diag_ref[7 * s + m, pl.ds(r, 8), :] = words(
                    _lincomb([(c, ops[k]) for k, c in a.items()]))


def _kernel(x_hbm, w_hbm, b_hbm, o_hbm, xbuf, obuf, wbuf, bbuf,
            wt_ref, plain_ref, diag_ref, bias_ref, isem, fsem, osem, wsem):
    NB, NK, _, S = x_hbm.shape
    F = w_hbm.shape[1]

    def istart(b, piece, priority):
        at = (b, slice(None), pl.ds(piece[0], 8), pl.ds(*piece[1:]))
        pltpu.make_async_copy(x_hbm.at[at], xbuf.at[at], isem.at[b]).start(priority=priority)

    def iwait(b):
        pltpu.make_async_copy(x_hbm.at[b], xbuf.at[b], isem.at[b]).wait()

    def fcopy(j):
        at = (0, slice(None), slice(None), pl.ds(j * CHUNK, CHUNK))
        return pltpu.make_async_copy(x_hbm.at[at], xbuf.at[at], fsem.at[j])

    def oslot(b):
        return jnp.where(b >= OUT_SLOTS, b - OUT_SLOTS, b)

    def ostart(b, pieces):
        slot = oslot(b)
        for piece in pieces:
            at = (slice(None), pl.ds(piece[0], 8), pl.ds(*piece[1:]))
            pltpu.make_async_copy(obuf.at[(slot, *at)], o_hbm.at[(b, *at)], osem.at[b]).start()

    def owait(b):
        pltpu.make_async_copy(obuf.at[oslot(b)], o_hbm.at[b], osem.at[b]).wait()

    def wcopy(j, blocks=4):
        rows = pl.ds(pl.multiple_of(j * 4 * KU, 4 * KU), blocks * KU)
        return pltpu.make_async_copy(w_hbm.at[rows], wbuf.at[rows], wsem.at[j])

    bcopy = pltpu.make_async_copy(b_hbm, bbuf, wsem.at[3])
    bcopy.start()
    wcopy(2, 1).start()
    wcopy(0).start()
    wcopy(1).start()
    bcopy.wait()
    bias = jnp.broadcast_to(bbuf[...].reshape(1, F).astype(jnp.float32), (128, F)).T
    for i in range(2):
        bias_ref[i] = jnp.concatenate(
            [bias[k + i * KU // 2:k + (i + 1) * KU // 2] for k in range(0, F, KU)], axis=0)
    wcopy(2, 1).wait()
    ninth, = _pruned_blocks(wbuf[8 * KU:, :])
    wt_ref[4] = _transposed(ninth, ninth)

    @pl.loop(0, 2)
    def _(j):
        @pl.when(j == 0)
        def _():
            for c in range(S // CHUNK):
                fcopy(c).start(priority=int(c >= 2))

        wcopy(j).wait()
        u = _pruned_blocks(wbuf[pl.ds(pl.multiple_of(j * 4 * KU, 4 * KU), 4 * KU), :])
        for e in range(2):
            wt_ref[2 * j + e] = _transposed(u[e], u[e + 2])

    _left_operands(wt_ref, plain_ref, diag_ref)

    def xblock(i, o, k, j):
        return xbuf[i, k, :, pl.ds(o + 128 * j, 128)]

    def right(i, o, b0, b1):
        return jnp.concatenate(
            [_lincomb([(c, xblock(i, o, *kj).astype(jnp.float32)) for kj, c in t.items()])
             for t in (b0, b1)], axis=0)

    def matmul(words, rhs):
        return jnp.dot(pltpu.bitcast(words, jnp.bfloat16), rhs.astype(jnp.bfloat16),
                       preferred_element_type=jnp.float32)

    def plain_round(i, slot, o, n, acc):
        ms = []
        for q, (_, (_, b0), (_, b1)) in enumerate(_PLAIN[n]):
            if len(b0) == len(b1) == 1:
                rhs = jnp.concatenate([xblock(i, o, *min(b0)), xblock(i, o, *min(b1))], axis=0)
            else:
                rhs = right(i, o, b0, b1)
            ms.append(matmul(plain_ref[4 * n + q], rhs))
        for c in ((0, 0), (0, 1), (1, 0), (1, 1)):
            terms = [(t[0][c], v) for t, v in zip(_PLAIN[n], ms) if c in t[0]]
            if not terms:
                continue
            acc[c] = _lincomb(terms, acc[c] if c in acc else bias_ref[c[0]])
            if not any(c in t[0] for rnd in _PLAIN[n + 1:] for t in rnd):
                obuf[slot, :, pl.ds(KU // 2 * c[0], KU // 2), pl.ds(o + 128 * c[1], 128)] = (
                    acc[c].astype(obuf.dtype).reshape(NK, KU // 2, 128))

    def diagonal_round(i, o, products, accs, rights):
        ms = []
        for g, s, m in products:
            for h, p in _STRASSEN[m][1]:
                if (g, s, h, p) not in rights:
                    (_, b0), (_, b1) = _DIAGONAL[s][h]
                    rights[g, s, h, p] = right(i, o + PAIR * (2 * g + p), b0, b1)
            rhs = _lincomb([(c, rights[g, s, h, p]) for (h, p), c in _STRASSEN[m][1].items()])
            ms.append(matmul(diag_ref[7 * s + m], rhs))
        n = F // 4
        for g, s in sorted({t[:2] for t in products}):
            for p in range(2):
                terms = [[(_STRASSEN[t[2]][2][q, p], v) for t, v in zip(products, ms)
                          if t[:2] == (g, s) and (q, p) in _STRASSEN[t[2]][2]] for q in range(2)]
                if any(terms):
                    acc = accs[2 * g + p]
                    prev = acc[s, s] if (s, s) in acc else bias_ref[s]
                    acc[s, s] = jnp.concatenate(
                        [_lincomb(terms[q], prev[n * q:n * q + n]) for q in range(2)], axis=0)

    reads = ([(0, o, 128) for o in range(0, S, 128)],
             [(r, o, CHUNK) for r in range(8, KU, 8) for o in range(0, S, CHUNK)])
    writes = [(r, o, CHUNK) for r in range(0, KU, 8) for o in range(0, S, CHUNK)]
    steady = NB - len(OUT_LAST)
    assert WRITE_LEAD <= len(writes) and len(OUT_LAST) >= 2
    last = [(steady + e, sum(sizes[:j + 1]), (r, c, min(CHUNK, n)))
            for e, sizes in enumerate(OUT_LAST) for j, n in enumerate(sizes)
            for r in range(0, KU, 8)
            for c in range(sum(sizes[:j]), sum(sizes[:j + 1]), CHUNK)]
    read_steps = S // (4 * PAIR) * _READS.count("1")
    write_steps = S // (4 * PAIR) * _WRITES.count("1")

    def share(pieces, step, steps):
        return range(step * 2 * len(pieces) // steps, (step + 1) * 2 * len(pieces) // steps)

    last_writes = {}
    position = steady * len(writes)
    for i in range(steady, NB):
        done = wstep = 0
        for t, kind in enumerate(S // (4 * PAIR) * _ROUNDS):
            done += PAIR * (kind == "c")
            if _WRITES[t % len(_ROUNDS)] == "1":
                due = ((2 * i - NB) * len(writes) + WRITE_LEAD
                       + share(writes, wstep, write_steps).stop)
                now = last_writes[i, wstep] = []
                while last and position < due and last[0][:2] <= (i, done) and len(now) < 12:
                    b, _, piece = last.pop(0)
                    now.append((b, piece))
                    position += piece[2] / CHUNK
                wstep += 1

    @pl.loop(0, NB)
    def _(i):
        @pl.when(i > 0)
        def _():
            iwait(i)

        @pl.when(i >= OUT_SLOTS)
        def _():
            owait(i - OUT_SLOTS)

        slot = oslot(i)
        ready = rstep = wstep = 0
        for o in range(0, S, 4 * PAIR):
            accs = [{} for _ in range(4)]
            rights = {}
            for t, kind in enumerate(_ROUNDS):
                k = _ROUNDS[:t].count(kind)
                products = _PRODUCTS[4 * k:4 * k + 4]
                pairs = (2 * products[-1][0] + 2 if kind == "d"
                         else k + 3 if kind == "c" else k + 1)
                while ready * CHUNK < min(o + PAIR * pairs, S):
                    @pl.when(i == 0)
                    def _():
                        fcopy(ready).wait()
                    ready += 1

                if kind == "d":
                    diagonal_round(i, o, products, accs, rights)
                else:
                    plain_round(i, slot, o + PAIR * k, "abc".index(kind), accs[k])

                if _READS[t] == "1":
                    for priority, pieces in enumerate(reads):
                        for q in share(pieces, rstep, read_steps):
                            db, q = divmod(q - READ_DELAY[priority], len(pieces))
                            b = 2 * i + 1 + db

                            @pl.when((b >= 1) & (b < NB))
                            def _():
                                istart(b, pieces[q], priority)
                    rstep += 1
                if _WRITES[t] == "1":
                    qs = [divmod(q + WRITE_LEAD, len(writes))
                          for q in share(writes, wstep, write_steps)]
                    for db in sorted({d for d, _ in qs}):
                        b = 2 * i - NB + db

                        @pl.when((b >= 0) & (b < steady))
                        def _():
                            ostart(b, [writes[q] for d, q in qs if d == db])
                    for it in range(steady, NB):
                        if last_writes[it, wstep]:
                            @pl.when(i == it)
                            def _():
                                for b, piece in last_writes[it, wstep]:
                                    ostart(b, [piece])
                    wstep += 1

    for b, _, piece in last:
        ostart(b, [piece])
    for b in range(NB - OUT_SLOTS, NB):
        owait(b)


@jax.jit
def pallas_standalone__structured_sparse_n_m__ragged_kernel(
    x: jax.Array,
    w: jax.Array,
    b: jax.Array,
):
    B, S, D = x.shape
    F = w.shape[1]
    xt = jnp.transpose(x, (0, 2, 1)).reshape(B, D // KU, KU, S)
    out = pl.pallas_call(
        _kernel,
        in_specs=[pl.BlockSpec(memory_space=pl.ANY)] * 3,
        out_specs=pl.BlockSpec(memory_space=pl.ANY),
        out_shape=jax.ShapeDtypeStruct((B, F // KU, KU, S), x.dtype),
        scratch_shapes=[
            pltpu.VMEM((B, D // KU, KU, S), x.dtype),
            pltpu.VMEM((OUT_SLOTS, F // KU, KU, S), x.dtype),
            pltpu.VMEM((D, F), w.dtype),
            pltpu.VMEM((F,), b.dtype),
            pltpu.VMEM((5, F // 2, 128), jnp.int32),
            pltpu.VMEM((12, F // 4, 128), jnp.int32),
            pltpu.VMEM((14, F // 8, 128), jnp.int32),
            pltpu.VMEM((2, F // 2, 128), jnp.float32),
            pltpu.SemaphoreType.DMA((B,)),
            pltpu.SemaphoreType.DMA((S // CHUNK,)),
            pltpu.SemaphoreType.DMA((B,)),
            pltpu.SemaphoreType.DMA((4,)),
        ],
        compiler_params=pltpu.CompilerParams(
            vmem_limit_bytes=120 * 1024 * 1024,
            disable_bounds_checks=True,
            disable_semaphore_checks=True,
            flags={"XLA_TPU_RESCHEDULE_DMA_DONES": True},
        ),
    )(xt, w, b)
    return jnp.transpose(out.reshape(B, F, S), (0, 2, 1))
```

```python
import jax
import jax.numpy as jnp
from jax import lax
import jax.experimental.pallas as pl
import jax.experimental.pallas.tpu as pltpu

KU = 64
PAIR = 256
OUT_SLOTS = 5

_T = 1.0 / 3.0
_PLAIN = (
    (({(0, 0): 1, (0, 1): -1},
      ({(0, 0): 1, (0, 1): -1}, {(1, 1): 1}), ({(0, 6): 1, (0, 7): -1}, {(7, 1): 1})),
     ({(0, 0): 1, (0, 1): -.5},
      ({(0, 4): 2, (0, 5): -2}, {(5, 1): 1}), ({(0, 2): 2, (0, 3): -2}, {(3, 1): 1})),
     ({(1, 0): 1, (1, 1): -1},
      ({(1, 0): 1, (1, 1): -1}, {(0, 0): 1}), ({(1, 6): 1, (1, 7): -1}, {(6, 0): 1})),
     ({(1, 0): 1, (1, 1): -.5},
      ({(1, 4): 1, (1, 5): -1}, {(4, 0): 1}), ({(1, 2): 1, (1, 3): -1}, {(2, 0): 1}))),
    (({(0, 0): 1, (1, 0): 1},
      ({(1, 1): 1}, {(0, 0): 1, (1, 0): 1}), ({(1, 5): 1}, {(4, 0): 1, (5, 0): 1})),
     ({(0, 0): 1, (1, 0): 2},
      ({(0, 8): -_T, (1, 8): 2 * _T}, {(8, 0): 1}), ({(1, 3): .5}, {(2, 0): 1, (3, 0): 1})),
     ({(0, 0): 1, (1, 0): .5},
      ({(0, 8): 4 * _T, (1, 8): -2 * _T}, {(8, 0): 1}), ({(1, 7): 2}, {(6, 0): 1, (7, 0): 1})),
     ({(0, 0): 1, (1, 1): 1},
      ({(0, 0): 1, (1, 1): -1}, {(0, 0): 1, (1, 1): -1}),
      ({(0, 2): 1, (1, 3): -.5}, {(2, 0): 1, (3, 1): -2}))),
    (({(0, 1): 1, (1, 1): 1},
      ({(0, 0): 1}, {(0, 1): 1, (1, 1): 1}), ({(0, 4): 1}, {(4, 1): 1, (5, 1): 1})),
     ({(0, 1): 1, (1, 1): 2},
      ({(0, 8): -_T, (1, 8): 2 * _T}, {(8, 1): 1}), ({(0, 2): 1}, {(2, 1): 1, (3, 1): 1})),
     ({(0, 1): 1, (1, 1): .5},
      ({(0, 8): 4 * _T, (1, 8): -2 * _T}, {(8, 1): 1}), ({(0, 6): 1}, {(6, 1): 1, (7, 1): 1})),
     ({(0, 0): 1, (1, 1): .5},
      ({(0, 4): 1, (1, 5): -1}, {(4, 0): 1, (5, 1): -2}),
      ({(0, 6): 1, (1, 7): -2}, {(6, 0): 1, (7, 1): -1}))),
)
_DIAGONAL = (
    ((({(0, 1): 1, (1, 1): -1}, {(1, 0): 1, (1, 1): 1}),
      ({(0, 3): 1, (1, 3): -.5}, {(3, 0): 1, (3, 1): 2})),
     (({(0, 5): 1, (1, 5): -1}, {(5, 0): 1, (5, 1): 2}),
      ({(0, 7): 1, (1, 7): -2}, {(7, 0): 1, (7, 1): 1}))),
    ((({(0, 0): -1, (1, 0): 1}, {(0, 0): 1, (0, 1): 1}),
      ({(0, 2): -1, (1, 2): .5}, {(2, 0): 1, (2, 1): 2})),
     (({(0, 4): -.5, (1, 4): .5}, {(4, 0): 1, (4, 1): 2}),
      ({(0, 6): -.5, (1, 6): 1}, {(6, 0): 1, (6, 1): 1}))),
)
_STRASSEN = (
    ({(0, 0): 1, (1, 1): 1}, {(0, 0): 1, (1, 1): 1}, {(0, 0): 1, (1, 1): 1}),
    ({(1, 1): 1}, {(1, 0): 1, (0, 0): -1}, {(0, 0): 1, (1, 0): 1}),
    ({(0, 0): 1, (0, 1): 1}, {(1, 1): 1}, {(0, 0): -1, (0, 1): 1}),
    ({(0, 1): 1, (1, 1): -1}, {(1, 0): 1, (1, 1): 1}, {(0, 0): 1}),
    ({(1, 0): 1, (1, 1): 1}, {(0, 0): 1}, {(1, 0): 1, (1, 1): -1}),
    ({(0, 0): 1}, {(0, 1): 1, (1, 1): -1}, {(0, 1): 1, (1, 1): 1}),
    ({(1, 0): 1, (0, 0): -1}, {(0, 0): 1, (0, 1): 1}, {(1, 1): 1}),
)
_PRODUCTS = [(g, s, m) for g in range(2) for ms in (range(5), (5, 6))
             for s in range(2) for m in ms]
_WHERE = {0: (0, 0), 1: (1, 0), 2: (0, 1), 3: (1, 1),
          4: (2, 0), 5: (3, 0), 6: (2, 1), 7: (3, 1), 8: (4, None)}

_ROUNDS = "adddbcdabcddabcdabc"
_READS = "1101111111011110111"
_WRITES = "0001001100010001100"

CHUNK = 512
WRITE_LEAD = 20
LAST_WRITES = (((None, (2048, 2048)),),
               ((0, (4096,)), (1, (2048, 1024, 1024))))


def _lincomb(terms, acc=None):
    for mag in sorted({abs(c) for c, _ in terms}, key=lambda m: (m != 1, m)):
        grp = sorted([(c, v) for c, v in terms if abs(c) == mag], key=lambda t: -t[0])
        if mag == 1 and acc is not None:
            for c, v in grp:
                acc = acc + v if c > 0 else acc - v
            continue
        sgn = 1 if grp[0][0] > 0 else -1
        s = grp[0][1]
        for c, v in grp[1:]:
            s = s + v if c * sgn > 0 else s - v
        if mag != 1:
            s = s * mag
        if acc is None:
            acc = s if sgn > 0 else -s
        else:
            acc = acc + s if sgn > 0 else acc - s
    return acc


def _prune_words(u):
    mate = lax.broadcasted_iota(jnp.int32, u.shape, 0) ^ 1
    lo = pltpu.bitcast((u << 16) & 0x7FFFFFFF, jnp.float32)
    hi = pltpu.bitcast(u & 0x7FFF0000, jnp.float32)
    big, small = jnp.maximum(lo, hi), jnp.minimum(lo, hi)
    nbig = jnp.take_along_axis(big, mate, axis=0, mode="promise_in_bounds")
    nsmall = jnp.take_along_axis(small, mate, axis=0, mode="promise_in_bounds")
    thr = jnp.maximum(jnp.minimum(big, nbig), jnp.maximum(small, nsmall))
    return u & (jnp.where(lo < thr, 0, 0xFFFF) | jnp.where(hi < thr, 0, -65536))


def _pruned_blocks(w):
    u = pltpu.bitcast(w, jnp.int32)
    return [jnp.concatenate([_prune_words(u[r:r + 8]) for r in range(k, k + KU // 2, 8)], axis=0)
            for k in range(0, u.shape[0], KU // 2)]


def _transposed(lo, hi):
    t = pltpu.bitcast(jnp.concatenate([lo, hi], axis=0), jnp.bfloat16)
    return pltpu.bitcast(t.T, jnp.int32)


def _left_operands(wt_ref, plain_ref, diag_ref):
    low = lax.broadcasted_iota(jnp.int32, (1, 128), 1) < KU

    def block(r, i, k, side):
        t, pos = _WHERE[k]
        v = wt_ref[t, pl.ds(r // 16 * 32 + 16 * i + r % 16, 8), :]
        return v if pos in (side, None) else pltpu.roll(v, KU, 1)

    def operand(r, a0, a1):
        acc = None
        for i in range(2):
            s0, s1 = ([k for k in sorted(a) if k[0] == i] for a in (a0, a1))
            for q in range(max(len(s0), len(s1))):
                c0 = a0[s0[q]] if q < len(s0) else 0
                c1 = a1[s1[q]] if q < len(s1) else 0
                if not (c0 and c1):
                    v = block(r, *s0[q], 0) if c0 else block(r, *s1[q], 1)
                elif _WHERE[s0[q][1]] == (_WHERE[s1[q][1]][0], 0):
                    v = block(r, *s0[q], 0)
                else:
                    v = jnp.where(low, block(r, *s0[q], 0), block(r, *s1[q], 1))
                v = pltpu.bitcast(v, jnp.bfloat16).astype(jnp.float32)
                if c0 == c1:
                    acc = _lincomb([(c0, v)], acc)
                else:
                    acc = _lincomb([(1, v * jnp.where(low, float(c0), float(c1)))], acc)
        return acc

    def store(ref, p, r, v):
        ref[pl.ds(r, 8), pl.ds(128 * p, 128)] = pltpu.bitcast(v.astype(jnp.bfloat16), jnp.int32)

    n = diag_ref.shape[0]
    for r in range(0, n, 8):
        for q in range(2):
            for p, (_, (a0, _), (a1, _)) in enumerate(t for rnd in _PLAIN for t in rnd):
                store(plain_ref, p, n * q + r, operand(n * q + r, a0, a1))
        for s, passes in enumerate(_DIAGONAL):
            ops = {(q, h): operand(n * q + r, a0, a1)
                   for q in range(2) for h, ((a0, _), (a1, _)) in enumerate(passes)}
            for m, (a, _, _) in enumerate(_STRASSEN):
                store(diag_ref, 7 * s + m, r, _lincomb([(c, ops[k]) for k, c in a.items()]))


def _pieces(u, rows, width, lo, hi):
    pieces = []
    for r in rows:
        split = 5 if r < KU else 4
        k0, k1 = (0, 9) if u is None else (0, split) if u == 0 else (split, 9)
        n = min(width, hi - lo)
        assert (hi - lo) % n == 0
        pieces += [((k0, k1 - k0), (r, 8), (o, n)) for o in range(lo, hi, n)]
    return pieces


def _share(n, step, steps):
    return range(step * n // steps, (step + 1) * n // steps)


def _plan_last_writes(slabs, tokens, writes, steps):
    first = slabs - len(LAST_WRITES)
    todo = [(first + e, tokens * (u != 0) + sum(sizes[:j + 1]), piece)
            for e, parts in enumerate(LAST_WRITES) for u, sizes in parts
            for j in range(len(sizes))
            for piece in _pieces(u, range(0, 2 * KU, 8), 1024,
                                 sum(sizes[:j]), sum(sizes[:j + 1]))]
    plan, position = {}, first * writes
    for m in range(first, slabs):
        done = step = 0
        for t, kind in enumerate(2 * tokens // (4 * PAIR) * _ROUNDS):
            done += PAIR * (kind == "c")
            if _WRITES[t % len(_ROUNDS)] == "1":
                due = (2 * m - slabs) * writes + WRITE_LEAD + _share(2 * writes, step, steps).stop
                now = plan[m, step] = []
                while todo and position < due and todo[0][:2] <= (m, done) and len(now) < 12:
                    d, _, piece = todo.pop(0)
                    now.append((d, piece))
                    position += piece[0][1] * piece[2][1] / (9 * 1024)
                step += 1
    return plan, [(d, piece) for d, _, piece in todo]


def _kernel(x_hbm, w_hbm, b_hbm, o_hbm, xbuf, obuf, wbuf, bbuf,
            wt_ref, plain_ref, diag_ref, bias_ref, isem, fsem, osem, wsem):
    slabs, _, _, S = x_hbm.shape
    F = w_hbm.shape[1]

    def read(d, piece, sem):
        at = (d, *(pl.ds(*p) for p in piece))
        return pltpu.make_async_copy(x_hbm.at[at], xbuf.at[at], sem)

    def first_reads(c):
        cols = (c * CHUNK, CHUNK)
        return [read(0, ((0, 4), (0, 2 * KU), cols), fsem.at[c]),
                read(0, ((4, 1), (0, KU), cols), fsem.at[c])]

    def oslot(d):
        return jnp.where(d >= OUT_SLOTS, d - OUT_SLOTS, d)

    def write(d, pieces):
        slot = oslot(d)
        for piece in pieces:
            at = [pl.ds(*p) for p in piece]
            pltpu.make_async_copy(obuf.at[(slot, *at)], o_hbm.at[(d, *at)], osem.at[d]).start()

    def wait_writes(d):
        pltpu.make_async_copy(obuf.at[oslot(d)], o_hbm.at[d], osem.at[d]).wait()

    def wcopy(j, blocks=4):
        rows = pl.ds(pl.multiple_of(j * 4 * KU, 4 * KU), blocks * KU)
        return pltpu.make_async_copy(w_hbm.at[rows], wbuf.at[rows], wsem.at[j])

    bcopy = pltpu.make_async_copy(b_hbm, bbuf, wsem.at[3])
    bcopy.start()
    wcopy(2, 1).start()
    wcopy(0).start()
    wcopy(1).start()
    bcopy.wait()
    bias = jnp.broadcast_to(bbuf[...].reshape(1, F).astype(jnp.float32), (128, F)).T
    for i in range(2):
        bias_ref[i] = jnp.concatenate(
            [bias[k + i * KU // 2:k + (i + 1) * KU // 2] for k in range(0, F, KU)], axis=0)
    wcopy(2, 1).wait()
    ninth, = _pruned_blocks(wbuf[8 * KU:, :])
    wt_ref[4] = _transposed(ninth, ninth)

    @pl.loop(0, 2)
    def _(j):
        @pl.when(j == 0)
        def _():
            for c in range(S // CHUNK):
                for copy in first_reads(c):
                    copy.start(priority=int(c >= 2))

        wcopy(j).wait()
        u = _pruned_blocks(wbuf[pl.ds(pl.multiple_of(j * 4 * KU, 4 * KU), 4 * KU), :])
        for e in range(2):
            wt_ref[2 * j + e] = _transposed(u[e], u[e + 2])

    _left_operands(wt_ref, plain_ref, diag_ref)

    def block(at, k, j, r=0, rows=KU):
        d, u, o = at
        g = F // KU * u + k
        return d, g // 2, pl.ds(g % 2 * KU + r, rows), pl.ds(o + 128 * j, 128)

    def right(at, b0, b1):
        return jnp.concatenate(
            [_lincomb([(c, xbuf[block(at, *kj)].astype(jnp.float32)) for kj, c in t.items()])
             for t in (b0, b1)], axis=0)

    def matmul(ref, p, rhs):
        lhs = pltpu.bitcast(ref[:, pl.ds(128 * p, 128)], jnp.bfloat16)
        return jnp.dot(lhs, rhs.astype(jnp.bfloat16), preferred_element_type=jnp.float32)

    def plain_round(at, slot, n, acc):
        ms = []
        for q, (_, (_, b0), (_, b1)) in enumerate(_PLAIN[n]):
            if len(b0) == len(b1) == 1:
                rhs = jnp.concatenate([xbuf[block(at, *min(t))] for t in (b0, b1)], axis=0)
            else:
                rhs = right(at, b0, b1)
            ms.append(matmul(plain_ref, 4 * n + q, rhs))
        for c in ((0, 0), (0, 1), (1, 0), (1, 1)):
            terms = [(t[0][c], v) for t, v in zip(_PLAIN[n], ms) if c in t[0]]
            if not terms:
                continue
            acc[c] = _lincomb(terms, acc[c] if c in acc else bias_ref[c[0]])
            if not any(c in t[0] for rnd in _PLAIN[n + 1:] for t in rnd):
                out, h = acc[c].astype(obuf.dtype), KU // 2
                for k in range(F // KU):
                    obuf[block((slot, *at[1:]), k, c[1], h * c[0], h)] = out[h * k:h * k + h]

    def diagonal_round(at, products, accs, rights):
        ms = []
        for g, s, m in products:
            for h, p in _STRASSEN[m][1]:
                if (g, s, h, p) not in rights:
                    (_, b0), (_, b1) = _DIAGONAL[s][h]
                    rights[g, s, h, p] = right((*at[:2], at[2] + PAIR * (2 * g + p)), b0, b1)
            rhs = _lincomb([(c, rights[g, s, h, p]) for (h, p), c in _STRASSEN[m][1].items()])
            ms.append(matmul(diag_ref, 7 * s + m, rhs))
        n = F // 4
        for g, s in sorted({t[:2] for t in products}):
            for p in range(2):
                terms = [[(_STRASSEN[t[2]][2][q, p], v) for t, v in zip(products, ms)
                          if t[:2] == (g, s) and (q, p) in _STRASSEN[t[2]][2]] for q in range(2)]
                if any(terms):
                    acc = accs[2 * g + p]
                    prev = acc[s, s] if (s, s) in acc else bias_ref[s]
                    acc[s, s] = jnp.concatenate(
                        [_lincomb(terms[q], prev[n * q:n * q + n]) for q in range(2)], axis=0)

    reads = (_pieces(None, range(0, 16, 8), 128, 0, S),
             _pieces(None, range(16, 2 * KU, 8), 512, 0, S))
    second = (_pieces(1, range(0, 16, 8), 256, 0, S),
              _pieces(1, range(16, 2 * KU, 8), 1024, 0, S))
    writes = _pieces(None, range(0, 2 * KU, 8), 1024, 0, S)
    read_steps = 2 * S // (4 * PAIR) * _READS.count("1")
    write_steps = 2 * S // (4 * PAIR) * _WRITES.count("1")
    steady = slabs - len(LAST_WRITES)
    assert WRITE_LEAD <= len(writes) and len(LAST_WRITES) >= 2
    planned, rest = _plan_last_writes(slabs, S, len(writes), write_steps)

    def read_step(m, step):
        for priority, pieces in enumerate(reads):
            for q in _share(2 * len(pieces), step, read_steps):
                e, q = divmod(q + len(pieces) // 2, len(pieces))
                d = 2 * m + e

                @pl.when((d >= 1) & (d < slabs))
                def _():
                    read(d, pieces[q], isem.at[d]).start(priority=priority)

            if step < read_steps // 4:
                @pl.when(m == 0)
                def _():
                    for q in _share(len(second[priority]), step, read_steps // 4):
                        read(0, second[priority][q], isem.at[0]).start(priority=priority)

    def write_step(m, step):
        qs = [divmod(q + WRITE_LEAD, len(writes))
              for q in _share(2 * len(writes), step, write_steps)]
        for e in sorted({e for e, _ in qs}):
            d = 2 * m - slabs + e

            @pl.when((d >= 0) & (d < steady))
            def _():
                write(d, [writes[q] for f, q in qs if f == e])

        for it in range(steady, slabs):
            if planned[it, step]:
                @pl.when(m == it)
                def _():
                    for d, piece in planned[it, step]:
                        write(d, [piece])

        if step == write_steps - 1:
            @pl.when((m + 1 >= OUT_SLOTS) & (m + 1 < slabs))
            def _():
                wait_writes(m + 1 - OUT_SLOTS)

    for copy in first_reads(0):
        copy.wait()

    @pl.loop(0, slabs)
    def _(m):
        slot = oslot(m)
        ready, rstep, wstep = 1, 0, 0
        for u, o in [(u, o) for u in range(2) for o in range(0, S, 4 * PAIR)]:
            accs = [{} for _ in range(4)]
            rights = {}
            for t, kind in enumerate(_ROUNDS):
                k = _ROUNDS[:t].count(kind)
                products = _PRODUCTS[4 * k:4 * k + 4]
                pairs = (2 * products[-1][0] + 2 if kind == "d"
                         else k + 3 if kind == "c" else k + 1)
                while ready * CHUNK < min(o + PAIR * pairs, S):
                    @pl.when(m == 0)
                    def _():
                        for copy in first_reads(ready):
                            copy.wait()
                    ready += 1

                if kind == "d":
                    diagonal_round((m, u, o), products, accs, rights)
                else:
                    plain_round((m, u, o + PAIR * k), slot, "abc".index(kind), accs[k])

                if _READS[t] == "1":
                    read_step(m, rstep)
                    rstep += 1
                if _WRITES[t] == "1":
                    write_step(m, wstep)
                    wstep += 1

            if (u, o) == (0, S - 4 * PAIR):
                @pl.when(m == 0)
                def _():
                    read(0, ((4, 1), (KU, KU), (0, S)), isem.at[0]).wait()
                    read(0, ((5, 4), (0, 2 * KU), (0, S)), isem.at[0]).wait()

        @pl.when(m + 1 < slabs)
        def _():
            pltpu.make_async_copy(x_hbm.at[m + 1], xbuf.at[m + 1], isem.at[m + 1]).wait()

    for d, piece in rest:
        write(d, [piece])
    for d in range(slabs - OUT_SLOTS, slabs):
        wait_writes(d)


@jax.jit
def pallas_standalone__structured_sparse_n_m__ragged_kernel(
    x: jax.Array,
    w: jax.Array,
    b: jax.Array,
):
    B, S, D = x.shape
    F = w.shape[1]
    assert D == F == 9 * KU
    slab = (D // KU, 2 * KU, S)
    xt = jnp.transpose(x, (0, 2, 1)).reshape(B // 2, *slab)
    out = pl.pallas_call(
        _kernel,
        in_specs=[pl.BlockSpec(memory_space=pl.ANY)] * 3,
        out_specs=pl.BlockSpec(memory_space=pl.ANY),
        out_shape=jax.ShapeDtypeStruct(xt.shape, x.dtype),
        scratch_shapes=[
            pltpu.VMEM(xt.shape, x.dtype),
            pltpu.VMEM((OUT_SLOTS, *slab), x.dtype),
            pltpu.VMEM((D, F), w.dtype),
            pltpu.VMEM((F,), b.dtype),
            pltpu.VMEM((5, F // 2, 128), jnp.int32),
            pltpu.VMEM((F // 4, 12 * 128), jnp.int32),
            pltpu.VMEM((F // 8, 14 * 128), jnp.int32),
            pltpu.VMEM((2, F // 2, 128), jnp.float32),
            pltpu.SemaphoreType.DMA((B // 2,)),
            pltpu.SemaphoreType.DMA((S // CHUNK,)),
            pltpu.SemaphoreType.DMA((B // 2,)),
            pltpu.SemaphoreType.DMA((4,)),
        ],
        compiler_params=pltpu.CompilerParams(
            vmem_limit_bytes=124 * 1024 * 1024,
            disable_bounds_checks=True,
            disable_semaphore_checks=True,
            flags={"XLA_TPU_RESCHEDULE_DMA_DONES": True},
        ),
    )(xt, w, b)
    return jnp.transpose(out.reshape(B, F, S), (0, 2, 1))
```

```python
import jax
import jax.numpy as jnp
from jax import lax
import jax.experimental.pallas as pl
import jax.experimental.pallas.tpu as pltpu

KU = 64
PAIR = 256
OUT_SLOTS = 5

_T = 1.0 / 3.0
_PLAIN = (
    (({(0, 0): 1, (0, 1): -1},
      ({(0, 0): 1, (0, 1): -1}, {(1, 1): 1}), ({(0, 6): 1, (0, 7): -1}, {(7, 1): 1})),
     ({(0, 0): 1, (0, 1): -.5},
      ({(0, 4): 2, (0, 5): -2}, {(5, 1): 1}), ({(0, 2): 2, (0, 3): -2}, {(3, 1): 1})),
     ({(1, 0): 1, (1, 1): -1},
      ({(1, 0): 1, (1, 1): -1}, {(0, 0): 1}), ({(1, 6): 1, (1, 7): -1}, {(6, 0): 1})),
     ({(1, 0): 1, (1, 1): -.5},
      ({(1, 4): 1, (1, 5): -1}, {(4, 0): 1}), ({(1, 2): 1, (1, 3): -1}, {(2, 0): 1}))),
    (({(0, 0): 1, (1, 0): 1},
      ({(1, 1): 1}, {(0, 0): 1, (1, 0): 1}), ({(1, 5): 1}, {(4, 0): 1, (5, 0): 1})),
     ({(0, 0): 1, (1, 0): 2},
      ({(0, 8): -_T, (1, 8): 2 * _T}, {(8, 0): 1}), ({(1, 3): .5}, {(2, 0): 1, (3, 0): 1})),
     ({(0, 0): 1, (1, 0): .5},
      ({(0, 8): 4 * _T, (1, 8): -2 * _T}, {(8, 0): 1}), ({(1, 7): 2}, {(6, 0): 1, (7, 0): 1})),
     ({(0, 0): 1, (1, 1): 1},
      ({(0, 0): 1, (1, 1): -1}, {(0, 0): 1, (1, 1): -1}),
      ({(0, 2): 1, (1, 3): -.5}, {(2, 0): 1, (3, 1): -2}))),
    (({(0, 1): 1, (1, 1): 1},
      ({(0, 0): 1}, {(0, 1): 1, (1, 1): 1}), ({(0, 4): 1}, {(4, 1): 1, (5, 1): 1})),
     ({(0, 1): 1, (1, 1): 2},
      ({(0, 8): -_T, (1, 8): 2 * _T}, {(8, 1): 1}), ({(0, 2): 1}, {(2, 1): 1, (3, 1): 1})),
     ({(0, 1): 1, (1, 1): .5},
      ({(0, 8): 4 * _T, (1, 8): -2 * _T}, {(8, 1): 1}), ({(0, 6): 1}, {(6, 1): 1, (7, 1): 1})),
     ({(0, 0): 1, (1, 1): .5},
      ({(0, 4): 1, (1, 5): -1}, {(4, 0): 1, (5, 1): -2}),
      ({(0, 6): 1, (1, 7): -2}, {(6, 0): 1, (7, 1): -1}))),
)
_DIAGONAL = (
    ((({(0, 1): 1, (1, 1): -1}, {(1, 0): 1, (1, 1): 1}),
      ({(0, 3): 2, (1, 3): -1}, {(3, 0): .5, (3, 1): 1})),
     (({(0, 5): 1, (1, 5): -1}, {(5, 0): 1, (5, 1): 2}),
      ({(0, 7): 1, (1, 7): -2}, {(7, 0): 1, (7, 1): 1}))),
    ((({(0, 0): -1, (1, 0): 1}, {(0, 0): 1, (0, 1): 1}),
      ({(0, 2): -1, (1, 2): .5}, {(2, 0): 1, (2, 1): 2})),
     (({(0, 4): -1, (1, 4): 1}, {(4, 0): .5, (4, 1): 1}),
      ({(0, 6): -.5, (1, 6): 1}, {(6, 0): 1, (6, 1): 1}))),
)
_STRASSEN = (
    ({(0, 0): 1, (1, 1): 1}, {(0, 0): 1, (1, 1): 1}, {(0, 0): 1, (1, 1): 1}),
    ({(1, 1): 1}, {(1, 0): 1, (0, 0): -1}, {(0, 0): 1, (1, 0): 1}),
    ({(0, 0): 1, (0, 1): 1}, {(1, 1): 1}, {(0, 0): -1, (0, 1): 1}),
    ({(0, 1): 1, (1, 1): -1}, {(1, 0): 1, (1, 1): 1}, {(0, 0): 1}),
    ({(1, 0): 1, (1, 1): 1}, {(0, 0): 1}, {(1, 0): 1, (1, 1): -1}),
    ({(0, 0): 1}, {(0, 1): 1, (1, 1): -1}, {(0, 1): 1, (1, 1): 1}),
    ({(1, 0): 1, (0, 0): -1}, {(0, 0): 1, (0, 1): 1}, {(1, 1): 1}),
)
_PRODUCTS = [(g, s, m) for g in range(2) for ms in (range(5), (5, 6))
             for s in range(2) for m in ms]
_WHERE = {0: (0, 0), 1: (1, 0), 2: (0, 1), 3: (1, 1),
          4: (2, 0), 5: (3, 0), 6: (2, 1), 7: (3, 1), 8: (4, None)}

_ROUNDS = "adddbcdabcddabcdabc"
_READS = "1101111111011110111"
_WRITES = "0001001100010001100"

CHUNK = 512
WRITE_LEAD = 20
LAST_WRITES = (((None, (2048, 2048)),),
               ((0, (4096,)), (1, (2048, 1024, 1024))))


def _lincomb(terms, acc=None):
    for mag in sorted({abs(c) for c, _ in terms}, key=lambda m: (m != 1, m)):
        grp = sorted([(c, v) for c, v in terms if abs(c) == mag], key=lambda t: -t[0])
        if mag == 1 and acc is not None:
            for c, v in grp:
                acc = acc + v if c > 0 else acc - v
            continue
        sgn = 1 if grp[0][0] > 0 else -1
        s = grp[0][1]
        for c, v in grp[1:]:
            s = s + v if c * sgn > 0 else s - v
        if mag != 1:
            s = s * mag
        if acc is None:
            acc = s if sgn > 0 else -s
        else:
            acc = acc + s if sgn > 0 else acc - s
    return acc


def _prune_words(u):
    mate = lax.broadcasted_iota(jnp.int32, u.shape, 0) ^ 1
    lo = pltpu.bitcast((u << 16) & 0x7FFFFFFF, jnp.float32)
    hi = pltpu.bitcast(u & 0x7FFF0000, jnp.float32)
    big, small = jnp.maximum(lo, hi), jnp.minimum(lo, hi)
    nbig = jnp.take_along_axis(big, mate, axis=0, mode="promise_in_bounds")
    nsmall = jnp.take_along_axis(small, mate, axis=0, mode="promise_in_bounds")
    thr = jnp.maximum(jnp.minimum(big, nbig), jnp.maximum(small, nsmall))
    return u & (jnp.where(lo < thr, 0, 0xFFFF) | jnp.where(hi < thr, 0, -65536))


def _pruned_blocks(w):
    u = pltpu.bitcast(w, jnp.int32)
    return [jnp.concatenate([_prune_words(u[r:r + 8]) for r in range(k, k + KU // 2, 8)], axis=0)
            for k in range(0, u.shape[0], KU // 2)]


def _transposed(lo, hi):
    t = pltpu.bitcast(jnp.concatenate([lo, hi], axis=0), jnp.bfloat16)
    return pltpu.bitcast(t.T, jnp.int32)


def _left_operands(wt_ref, plain_ref, diag_ref):
    low = lax.broadcasted_iota(jnp.int32, (1, 128), 1) < KU

    def block(r, i, k, side):
        t, pos = _WHERE[k]
        v = wt_ref[t, pl.ds(r // 16 * 32 + 16 * i + r % 16, 8), :]
        return v if pos in (side, None) else pltpu.roll(v, KU, 1)

    def operand(r, a0, a1):
        acc = None
        for i in range(2):
            s0, s1 = ([k for k in sorted(a) if k[0] == i] for a in (a0, a1))
            for q in range(max(len(s0), len(s1))):
                c0 = a0[s0[q]] if q < len(s0) else 0
                c1 = a1[s1[q]] if q < len(s1) else 0
                if not (c0 and c1):
                    v = block(r, *s0[q], 0) if c0 else block(r, *s1[q], 1)
                elif _WHERE[s0[q][1]] == (_WHERE[s1[q][1]][0], 0):
                    v = block(r, *s0[q], 0)
                else:
                    v = jnp.where(low, block(r, *s0[q], 0), block(r, *s1[q], 1))
                v = pltpu.bitcast(v, jnp.bfloat16).astype(jnp.float32)
                if c0 == c1:
                    acc = _lincomb([(c0, v)], acc)
                else:
                    acc = _lincomb([(1, v * jnp.where(low, float(c0), float(c1)))], acc)
        return acc

    def store(ref, p, r, v):
        ref[pl.ds(r, 8), pl.ds(128 * p, 128)] = pltpu.bitcast(v.astype(jnp.bfloat16), jnp.int32)

    n = diag_ref.shape[0]
    for r in range(0, n, 8):
        for q in range(2):
            for p, (_, (a0, _), (a1, _)) in enumerate(t for rnd in _PLAIN for t in rnd):
                store(plain_ref, p, n * q + r, operand(n * q + r, a0, a1))
        for s, passes in enumerate(_DIAGONAL):
            ops = {(q, h): operand(n * q + r, a0, a1)
                   for q in range(2) for h, ((a0, _), (a1, _)) in enumerate(passes)}
            for m, (a, _, _) in enumerate(_STRASSEN):
                store(diag_ref, 7 * s + m, r, _lincomb([(c, ops[k]) for k, c in a.items()]))


def _pieces(u, rows, width, lo, hi):
    pieces = []
    for r in rows:
        split = 5 if r < KU else 4
        k0, k1 = (0, 9) if u is None else (0, split) if u == 0 else (split, 9)
        n = min(width, hi - lo)
        assert (hi - lo) % n == 0
        pieces += [((k0, k1 - k0), (r, 8), (o, n)) for o in range(lo, hi, n)]
    return pieces


def _share(n, step, steps):
    return range(step * n // steps, (step + 1) * n // steps)


def _plan_last_writes(slabs, tokens, writes, steps):
    first = slabs - len(LAST_WRITES)
    todo = [(first + e, tokens * (u != 0) + sum(sizes[:j + 1]), piece)
            for e, parts in enumerate(LAST_WRITES) for u, sizes in parts
            for j in range(len(sizes))
            for piece in _pieces(u, range(0, 2 * KU, 8), 1024,
                                 sum(sizes[:j]), sum(sizes[:j + 1]))]
    plan, position = {}, first * writes
    for m in range(first, slabs):
        done = step = 0
        for t, kind in enumerate(2 * tokens // (4 * PAIR) * _ROUNDS):
            done += PAIR * (kind == "c")
            if _WRITES[t % len(_ROUNDS)] == "1":
                due = (2 * m - slabs) * writes + WRITE_LEAD + _share(2 * writes, step, steps).stop
                now = plan[m, step] = []
                while todo and position < due and todo[0][:2] <= (m, done) and len(now) < 12:
                    d, _, piece = todo.pop(0)
                    now.append((d, piece))
                    position += piece[0][1] * piece[2][1] / (9 * 1024)
                step += 1
    return plan, [(d, piece) for d, _, piece in todo]


def _kernel(x_hbm, w_hbm, b_hbm, o_hbm, xbuf, obuf, wbuf, bbuf,
            wt_ref, plain_ref, diag_ref, bias_ref, isem, fsem, osem, wsem):
    slabs, _, _, S = x_hbm.shape
    F = w_hbm.shape[1]

    def read(d, piece, sem):
        at = (d, *(pl.ds(*p) for p in piece))
        return pltpu.make_async_copy(x_hbm.at[at], xbuf.at[at], sem)

    def first_reads(c):
        cols = (c * CHUNK, CHUNK)
        return [read(0, ((0, 4), (0, 2 * KU), cols), fsem.at[c]),
                read(0, ((4, 1), (0, KU), cols), fsem.at[c])]

    middle = read(0, ((4, 1), (KU, KU), (0, S)), fsem.at[S // CHUNK])

    def oslot(d):
        return jnp.where(d >= OUT_SLOTS, d - OUT_SLOTS, d)

    def write(d, pieces):
        slot = oslot(d)
        for piece in pieces:
            at = [pl.ds(*p) for p in piece]
            pltpu.make_async_copy(obuf.at[(slot, *at)], o_hbm.at[(d, *at)], osem.at[d]).start()

    def wait_writes(d):
        pltpu.make_async_copy(obuf.at[oslot(d)], o_hbm.at[d], osem.at[d]).wait()

    def wcopy(j, blocks=4):
        rows = pl.ds(pl.multiple_of(j * 4 * KU, 4 * KU), blocks * KU)
        return pltpu.make_async_copy(w_hbm.at[rows], wbuf.at[rows], wsem.at[j])

    bcopy = pltpu.make_async_copy(b_hbm, bbuf, wsem.at[3])
    bcopy.start()
    wcopy(2, 1).start()
    wcopy(0).start()
    wcopy(1).start()
    bcopy.wait()
    bias = jnp.broadcast_to(bbuf[...].reshape(1, F).astype(jnp.float32), (128, F)).T
    for i in range(2):
        bias_ref[i] = jnp.concatenate(
            [bias[k + i * KU // 2:k + (i + 1) * KU // 2] for k in range(0, F, KU)], axis=0)
    wcopy(2, 1).wait()
    ninth, = _pruned_blocks(wbuf[8 * KU:, :])
    wt_ref[4] = _transposed(ninth, ninth)

    @pl.loop(0, 2)
    def _(j):
        @pl.when(j == 0)
        def _():
            for c in range(S // CHUNK):
                for copy in first_reads(c):
                    copy.start(priority=int(c >= 2))

        @pl.when(j == 1)
        def _():
            middle.start(priority=1)

        wcopy(j).wait()
        u = _pruned_blocks(wbuf[pl.ds(pl.multiple_of(j * 4 * KU, 4 * KU), 4 * KU), :])
        for e in range(2):
            wt_ref[2 * j + e] = _transposed(u[e], u[e + 2])

    _left_operands(wt_ref, plain_ref, diag_ref)

    def block(at, k, j, r=0, rows=KU):
        d, u, o = at
        g = F // KU * u + k
        return d, g // 2, pl.ds(g % 2 * KU + r, rows), pl.ds(o + 128 * j, 128)

    def right(at, b0, b1):
        return jnp.concatenate(
            [_lincomb([(c, xbuf[block(at, *kj)].astype(jnp.float32)) for kj, c in t.items()])
             for t in (b0, b1)], axis=0)

    def matmul(ref, p, rhs):
        lhs = pltpu.bitcast(ref[:, pl.ds(128 * p, 128)], jnp.bfloat16)
        return jnp.dot(lhs, rhs.astype(jnp.bfloat16), preferred_element_type=jnp.float32)

    def plain_round(at, slot, n, acc):
        ms = []
        for q, (_, (_, b0), (_, b1)) in enumerate(_PLAIN[n]):
            if len(b0) == len(b1) == 1:
                rhs = jnp.concatenate([xbuf[block(at, *min(t))] for t in (b0, b1)], axis=0)
            else:
                rhs = right(at, b0, b1)
            ms.append(matmul(plain_ref, 4 * n + q, rhs))
        for c in ((0, 0), (0, 1), (1, 0), (1, 1)):
            terms = [(t[0][c], v) for t, v in zip(_PLAIN[n], ms) if c in t[0]]
            if not terms:
                continue
            acc[c] = _lincomb(terms, acc[c] if c in acc else bias_ref[c[0]])
            if not any(c in t[0] for rnd in _PLAIN[n + 1:] for t in rnd):
                out, h = acc[c].astype(obuf.dtype), KU // 2
                for k in range(F // KU):
                    obuf[block((slot, *at[1:]), k, c[1], h * c[0], h)] = out[h * k:h * k + h]

    def diagonal_round(at, products, accs, rights):
        ms = []
        for g, s, m in products:
            for h, p in _STRASSEN[m][1]:
                if (g, s, h, p) not in rights:
                    (_, b0), (_, b1) = _DIAGONAL[s][h]
                    rights[g, s, h, p] = right((*at[:2], at[2] + PAIR * (2 * g + p)), b0, b1)
            rhs = _lincomb([(c, rights[g, s, h, p]) for (h, p), c in _STRASSEN[m][1].items()])
            ms.append(matmul(diag_ref, 7 * s + m, rhs))
        n = F // 4
        for g, s in sorted({t[:2] for t in products}):
            for p in range(2):
                terms = [[(_STRASSEN[t[2]][2][q, p], v) for t, v in zip(products, ms)
                          if t[:2] == (g, s) and (q, p) in _STRASSEN[t[2]][2]] for q in range(2)]
                if any(terms):
                    acc = accs[2 * g + p]
                    prev = acc[s, s] if (s, s) in acc else bias_ref[s]
                    acc[s, s] = jnp.concatenate(
                        [_lincomb(terms[q], prev[n * q:n * q + n]) for q in range(2)], axis=0)

    reads = (_pieces(None, range(0, 16, 8), 128, 0, S),
             _pieces(None, range(16, 2 * KU, 8), 512, 0, S))
    second = [[((5, 4), *piece[1:]) for piece in pieces]
              for pieces in (_pieces(1, range(0, 16, 8), 256, 0, S),
                             _pieces(1, range(16, 2 * KU, 8), 1024, 0, S))]
    writes = _pieces(None, range(0, 2 * KU, 8), 1024, 0, S)
    read_steps = 2 * S // (4 * PAIR) * _READS.count("1")
    write_steps = 2 * S // (4 * PAIR) * _WRITES.count("1")
    steady = slabs - len(LAST_WRITES)
    assert WRITE_LEAD <= len(writes) and len(LAST_WRITES) >= 2
    planned, rest = _plan_last_writes(slabs, S, len(writes), write_steps)

    def read_step(m, step):
        for priority, pieces in enumerate(reads):
            for q in _share(2 * len(pieces), step, read_steps):
                e, q = divmod(q + len(pieces) // 2, len(pieces))
                d = 2 * m + e

                @pl.when((d >= 1) & (d < slabs))
                def _():
                    read(d, pieces[q], isem.at[d]).start(priority=priority)

            if step < read_steps // 4:
                @pl.when(m == 0)
                def _():
                    for q in _share(len(second[priority]), step, read_steps // 4):
                        read(0, second[priority][q], isem.at[0]).start(priority=priority)

    def write_step(m, step):
        qs = [divmod(q + WRITE_LEAD, len(writes))
              for q in _share(2 * len(writes), step, write_steps)]
        for e in sorted({e for e, _ in qs}):
            d = 2 * m - slabs + e

            @pl.when((d >= 0) & (d < steady))
            def _():
                write(d, [writes[q] for f, q in qs if f == e])

        for it in range(steady, slabs):
            if planned[it, step]:
                @pl.when(m == it)
                def _():
                    for d, piece in planned[it, step]:
                        write(d, [piece])

        if step == write_steps - 1:
            @pl.when((m + 1 >= OUT_SLOTS) & (m + 1 < slabs))
            def _():
                wait_writes(m + 1 - OUT_SLOTS)

    for copy in first_reads(0):
        copy.wait()

    @pl.loop(0, slabs)
    def _(m):
        slot = oslot(m)
        ready, rstep, wstep = 1, 0, 0
        for u, o in [(u, o) for u in range(2) for o in range(0, S, 4 * PAIR)]:
            accs = [{} for _ in range(4)]
            rights = {}
            for t, kind in enumerate(_ROUNDS):
                k = _ROUNDS[:t].count(kind)
                products = _PRODUCTS[4 * k:4 * k + 4]
                pairs = (2 * products[-1][0] + 2 if kind == "d"
                         else k + 3 if kind == "c" else k + 1)
                while ready * CHUNK < min(o + PAIR * pairs, S):
                    @pl.when(m == 0)
                    def _():
                        for copy in first_reads(ready):
                            copy.wait()
                    ready += 1

                if kind == "d":
                    diagonal_round((m, u, o), products, accs, rights)
                else:
                    plain_round((m, u, o + PAIR * k), slot, "abc".index(kind), accs[k])

                if _READS[t] == "1":
                    read_step(m, rstep)
                    rstep += 1
                if _WRITES[t] == "1":
                    write_step(m, wstep)
                    wstep += 1

            if (u, o) == (0, S - 4 * PAIR):
                @pl.when(m == 0)
                def _():
                    middle.wait()
                    read(0, ((5, 4), (0, 2 * KU), (0, S)), isem.at[0]).wait()

        @pl.when(m + 1 < slabs)
        def _():
            pltpu.make_async_copy(x_hbm.at[m + 1], xbuf.at[m + 1], isem.at[m + 1]).wait()

    for d, piece in rest:
        write(d, [piece])
    for d in range(slabs - OUT_SLOTS, slabs):
        wait_writes(d)


@jax.jit
def pallas_standalone__structured_sparse_n_m__ragged_kernel(
    x: jax.Array,
    w: jax.Array,
    b: jax.Array,
):
    B, S, D = x.shape
    F = w.shape[1]
    assert D == F == 9 * KU
    slab = (D // KU, 2 * KU, S)
    xt = jnp.transpose(x, (0, 2, 1)).reshape(B // 2, *slab)
    out = pl.pallas_call(
        _kernel,
        in_specs=[pl.BlockSpec(memory_space=pl.ANY)] * 3,
        out_specs=pl.BlockSpec(memory_space=pl.ANY),
        out_shape=jax.ShapeDtypeStruct(xt.shape, x.dtype),
        scratch_shapes=[
            pltpu.VMEM(xt.shape, x.dtype),
            pltpu.VMEM((OUT_SLOTS, *slab), x.dtype),
            pltpu.VMEM((D, F), w.dtype),
            pltpu.VMEM((F,), b.dtype),
            pltpu.VMEM((5, F // 2, 128), jnp.int32),
            pltpu.VMEM((F // 4, 12 * 128), jnp.int32),
            pltpu.VMEM((F // 8, 14 * 128), jnp.int32),
            pltpu.VMEM((2, F // 2, 128), jnp.float32),
            pltpu.SemaphoreType.DMA((B // 2,)),
            pltpu.SemaphoreType.DMA((S // CHUNK + 1,)),
            pltpu.SemaphoreType.DMA((B // 2,)),
            pltpu.SemaphoreType.DMA((4,)),
        ],
        compiler_params=pltpu.CompilerParams(
            vmem_limit_bytes=124 * 1024 * 1024,
            disable_bounds_checks=True,
            disable_semaphore_checks=True,
            flags={"XLA_TPU_RESCHEDULE_DMA_DONES": True},
        ),
    )(xt, w, b)
    return jnp.transpose(out.reshape(B, F, S), (0, 2, 1))
```
